```python
import jax
import jax.numpy as jnp

def _softmax(x, axis=-1):
    return jax.nn.softmax(x, axis=axis)
def _gelu(x):
    return jax.nn.gelu(x, approximate=True)
def _silu(x):
    return jax.nn.silu(x)
def _sigmoid(x):
    return jax.nn.sigmoid(x)
def _layernorm(x, axis=-1, eps=1e-5):
    m = jnp.mean(x, axis=axis, keepdims=True)
    v = jnp.var(x, axis=axis, keepdims=True)
    return (x - m) / jnp.sqrt(v + eps)
def _scatter_add(tgt, idx, src, axis=0):
    return tgt.at[idx].add(src)
def _segment_sum(src, seg, n):
    return jax.ops.segment_sum(src, seg, n)
class _Rng:
    def __init__(self, key):
        self._k = key
    def _next(self):
        self._k, sub = jax.random.split(self._k)
        return sub
    def normal(self, shape):
        return jax.random.normal(self._next(), shape, dtype=jnp.bfloat16)
    def randint(self, lo, hi, shape):
        return jax.random.randint(self._next(), shape, lo, hi, dtype=jnp.int32)
    def uniform(self, shape, lo=0.0, hi=1.0):
        return jax.random.uniform(self._next(), shape, jnp.bfloat16, lo, hi)
    def permutation(self, n):
        return jax.random.permutation(self._next(), n)


kernel_name = 'gated_mix__sliding_block_cached__moe_arch_mod__decode'

def setup_inputs():
    _rng = _Rng(jax.random.key(int.from_bytes(__import__("os").urandom(4), "little")))
    _w = (lambda a: (lambda t: t.astype(jnp.bfloat16) if jnp.issubdtype(t.dtype, jnp.floating) else t)(jnp.asarray(a)))
    def _A_setup():
        B, Sq, D = 1, 1, 640
        Hq, Hkv, Sk, Dh = 32, 32, 32768, 192
        assert Hq % Hkv == 0, (Hq, Hkv)
        return {
            "x": _w((lambda *s: _rng.normal(s) * 0.05)(B, Sq, D)),
            "k_cache": _w((lambda *s: _rng.normal(s) * 0.05)(B, Hkv, Sk, Dh)),
            "v_cache": _w((lambda *s: _rng.normal(s) * 0.05)(B, Hkv, Sk, Dh)),
            "wq": _w((lambda *s: _rng.normal(s) * 0.05)(D, Hq * Dh) * (D ** -0.5)),
            "wo": _w((lambda *s: _rng.normal(s) * 0.05)(Hq * Dh, D) * ((Hq * Dh) ** -0.5)),
        }
    _A_in = _A_setup()

    def _B_setup():
        B, S, D, F, C = 1, 1, 640, 1536, 1
        return {
            "x": _w((lambda *s: _rng.normal(s) * 0.05)(B, S, D)),
            "w_r": _w((lambda *s: _rng.normal(s) * 0.05)(D)),
            "w_gate": _w((lambda *s: _rng.normal(s) * 0.05)(D, F)),
            "w_up": _w((lambda *s: _rng.normal(s) * 0.05)(D, F)),
            "w_down": _w((lambda *s: _rng.normal(s) * 0.05)(F, D)),
        }
    _B_in = _B_setup()

    return {
        "A_x": _A_in["x"],
        "A_k_cache": _A_in["k_cache"],
        "A_v_cache": _A_in["v_cache"],
        "A_wq": _A_in["wq"],
        "A_wo": _A_in["wo"],
        "B_x": _B_in["x"],
        "B_w_r": _B_in["w_r"],
        "B_w_gate": _B_in["w_gate"],
        "B_w_up": _B_in["w_up"],
        "B_w_down": _B_in["w_down"],
        "gate_w": _w((lambda *s: _rng.normal(s) * 0.05)(640)),
    }

def reference(A_x, A_k_cache, A_v_cache, A_wq, A_wo, B_x, B_w_r, B_w_gate, B_w_up, B_w_down, gate_w):
    def _A_ref(x, k_cache, v_cache, wq, wo):
        B, Sq, D = x.shape
        Hq, Dh = 32, 192
        Hkv, Sk = k_cache.shape[1], k_cache.shape[2]
        W = min(4096, max(256, Sk // 4))
        rep = Hq // Hkv
        q = (lambda x, *d: x.transpose(*d))((x @ wq).reshape(B, Sq, Hq, Dh), 0, 2, 1, 3)
        k = jnp.repeat(k_cache[:, :, Sk - W:, :], rep, axis=1)
        v = jnp.repeat(v_cache[:, :, Sk - W:, :], rep, axis=1)
        scores = jnp.einsum("bhqd,bhkd->bhqk", q, k) * (Dh ** -0.5)
        p = _softmax(scores, axis=-1)
        o = jnp.einsum("bhqk,bhkd->bhqd", p, v)
        return (lambda x, *d: x.transpose(*d))(o, 0, 2, 1, 3).reshape(B, Sq, Hq * Dh) @ wo

    def _B_ref(x, w_r, w_gate, w_up, w_down):
        B, S, D = x.shape
        C = 1
        r = x @ w_r
        idx = jnp.argsort(-r, axis=-1)[:, :C]
        idx_e = jnp.repeat(idx.reshape(B, C, 1), D, axis=2)
        x_sel = jnp.take_along_axis(x, idx_e, axis=1)
        g = _silu(x_sel @ w_gate)
        u = x_sel @ w_up
        y = (g * u) @ w_down
        r_sel = _sigmoid(jnp.take_along_axis(r, idx, axis=1))
        y = y * r_sel.reshape(B, C, 1)
        b_off = (jnp.arange(B) * S).reshape(B, 1)
        flat_idx = (idx + b_off).reshape(B * C)
        zero = (x * 0.0).reshape(B * S, D)
        upd = _scatter_add(zero, flat_idx, y.reshape(B * C, D), axis=0)
        return x + upd.reshape(B, S, D)

    x = A_x
    g = _sigmoid((x * gate_w).sum(-1, keepdims=True))
    a = _A_ref(x, A_k_cache, A_v_cache, A_wq, A_wo)
    b = _B_ref(x, B_w_r, B_w_gate, B_w_up, B_w_down)
    return g * a + (1 - g) * b
```

```python
import jax
import jax.numpy as jnp
import jax.experimental.pallas as pl
import jax.experimental.pallas.tpu as pltpu

H, DH, SK, D, F = 32, 192, 32768, 640, 1536
W = min(4096, max(256, SK // 4))
BASE = SK - W
M = 8
NP = H // 2
PD = 2 * DH
G = W // M
f32, bf16 = jnp.float32, jnp.bfloat16
A = (512, 1024, 1024, 1024, 512)

DEFAULT = dict(S=192, KR=(48, 24), cols=(512,) * 8, L=20, name="gated_mix_decode", prof=False, dly=0,
               qs=(5, 16), gs=(2, 20), os=4, pro0=12, prod=40, tw=14, last_end=72, comp=True, fast=24,
               tail0=128, tail=(128, 128, 64), vpu=(32, 32), gap=3, lgap=2, flags=None, tscr=2, t1end=8,
               corder=None, torder=None, t0end=120, xstart=74, VR=96)

SPLIT = [[(0, 0, 4)], [(0, 4, 1), (1, 0, 3)], [(1, 3, 2), (2, 0, 2)], [(2, 2, 3), (3, 0, 1)], [(3, 1, 4)]]


def _spread(n, t0, t1):
    return [t0 + int((i + 0.5) * (t1 - t0) / n) for i in range(n)]


def _sweep(k, stride):
    rgs = [b + o + stride * i for b in range(0, D // 8, k * stride) for o in range(stride) for i in range(k)]
    return [(rg, c) for g in range(0, D // 8, k) for c in range(2) for rg in rgs[g:g + k]]


def make(**kw):
    P = dict(DEFAULT)
    P.update(kw)
    S, cols, L = P['S'], P['cols'], P['L']
    cl = [(sum(cols[:i]), cols[i]) for i in range(len(cols))]
    if P['corder']:
        cl = [cl[i] for i in P['corder']]
    pcs = []
    Ss = S if isinstance(S, tuple) else (S,) * (PD // S)
    for w in range(2):
        for i, s in enumerate(Ss):
            r0 = sum(Ss[:i])
            for c, cw in cl:
                kr = P['KR'][0] if cw <= 512 else P['KR'][1]
                pcs += [(w, r, c, min(kr, r0 + s - r), cw) for r in range(r0, r0 + s, kr)]
    T = len(pcs)
    NS = min(s for s in range(L, T + 1) if T % s == 0)
    chunks = [P['tail0']] + list(P['tail']) + list(P['vpu'])
    assert sum(chunks) == 512
    n_mxu = 1 + len(P['tail'])
    comp = P['comp']
    sc_t = lambda t: t * T // 128

    def ready(w, a, g=None):
        return max(t for t, (w_, r, c, nr, nc) in enumerate(pcs)
                   if w_ == w and r < (a + 1) * DH and r + nr > a * DH and (g is None or (c < (g + 1) * G and c + nc > g * G)))

    def kern(x_hbm, kT, vT, wq, wo, wr_hbm, wg, wu, wd, gw_hbm, out_ref,
             x_v, wr_v, gw_v, w1_b, kv_b, wo_b, wd_b, q_s, o_s, oc_s, sems):
        def ds(start, n):
            return pl.ds(start if isinstance(start, int) else pl.multiple_of(start, n), n)

        def sem(i):
            return sems.at[NS + i]

        def kv(j, t):
            w, r, c, nr, nc = pcs[t]
            return pltpu.make_async_copy((kT, vT)[w].at[j, pl.ds(r, nr), pl.ds(BASE + c, nc)],
                                         kv_b.at[w, pl.ds(r, nr), pl.ds(c, nc)], sems.at[t % NS])

        def start0(*cs):
            for c in cs:
                c.start(priority=0)

        def wide(src, col, j, rg, c):
            return pltpu.make_async_copy(src.at[pl.ds(8 * rg, 8), ds(col, 512)],
                                         w1_b.at[j, c, pl.ds(8 * rg, 8)], sem(2 * (j % 2) + c))

        def u_q(j):
            return [lambda rg=rg, c=c: start0(wide(wq, j * 1024 + c * 512, j, rg, c)) for rg, c in _sweep(*P['qs'])]

        def u_g(j):
            return [lambda rg=rg, c=c: start0(wide((wg, wu)[c], (j - 6) * 512, j, rg, c)) for rg, c in _sweep(*P['gs'])]

        def tall(src, dst, blk, row, u, s):
            return [pltpu.make_async_copy(src.at[blk, pl.ds(row + 8 * rg, 8), pl.ds(128 * c, 128 * n)],
                                          dst.at[blk, pl.ds(row + 8 * rg, 8), pl.ds(128 * c, 128 * n)], s)
                    for rg, c, n in SPLIT[u]]

        def u_t(blocks, s):
            k = P['os']
            return [lambda b=b, row=row, u=u: start0(*tall(*b, row, u, s)) for g in range(0, 4, k)
                    for row in range(0, 256, 32) for u in range(5) for b in blocks[g:g + k]]

        def wait_all(bufs, s):
            for buf in bufs:
                pltpu.make_async_copy(buf, buf, s).wait()

        def stream(j, issue, tasks, gap, last=False, extra=()):
            at, t = {}, -gap
            for t0, fn in tasks:
                t = max(t + gap, t0)
                at.setdefault(min(t, T - 1), []).append(fn)
            t = P['xstart'] - 1
            for t0, fn in extra:
                t = max(t + 1, t0)
                at.setdefault(min(t, T - 1), []).append(fn)
            for t in range(T):
                kv(j, t).wait()
                for fn in issue.get(t, []):
                    fn()
                if t + L < T:
                    kv(j, t + L).start(priority=1)
                elif not last:
                    kv(j + 1, t + L - T).start(priority=1)
                if P['dly']:
                    pl.delay(P['dly'])
                for fn in at.get(t, []):
                    fn()

        if P['prof']:
            stream = jax.named_scope("grp")(stream)

        def trickle(units, t0, t1, issue=None):
            issue = {} if issue is None else issue
            for u, t in zip(units, _spread(len(units), t0, t1)):
                issue.setdefault(t, []).append(u)
            return issue

        row = jax.lax.broadcasted_iota(jnp.int32, (M, 1), 0)
        scale = DH ** -0.5

        def scores(st, j, a):
            def qk(g):
                if g == 0:
                    q = jnp.concatenate([q_s[3 * j + a + i] for i in range(2)], axis=1)
                    st['q'] = q[:, 64 * a:64 * a + DH].astype(bf16)
                s = jnp.dot(st['q'], kv_b[0, a * DH:(a + 1) * DH, g * G:(g + 1) * G], preferred_element_type=f32)
                st['s'] = s if g == 0 else jnp.where(row == g, s, st['s'])

            def softmax():
                del st['q']
                sc = st.pop('s') * scale
                m = jnp.max(jnp.max(sc, axis=1, keepdims=True), axis=0, keepdims=True)
                e = jnp.exp(sc - m)
                den = jnp.sum(jnp.sum(e, axis=1, keepdims=True), axis=0, keepdims=True)
                st['p%d' % a] = e / den
            return [(ready(0, a, g), lambda g=g: qk(g)) for g in range(M)] + [(0, softmax)] if comp else []

        def values(st, j, a, late=False):
            def pv(g):
                o = jax.lax.dot_general(st['p%d' % a].astype(bf16), kv_b[1, a * DH:(a + 1) * DH, g * G:(g + 1) * G],
                                        (((1,), (1,)), ((), ())), preferred_element_type=f32)
                st['o%d' % a] = o if g == 0 else jnp.where(row == g, o, st['o%d' % a])
                if g == M - 1:
                    del st['p%d' % a]
                    if a == 1:
                        o = jnp.concatenate([st.pop('o0'), st.pop('o1')], axis=1)
                        o = jnp.broadcast_to(jnp.sum(o, axis=0, keepdims=True), (M, PD))
                        for i in range(3):
                            o_s[3 * j + i] = o[:, 128 * i:128 * (i + 1)]
            return [(0 if late else ready(1, a, g), lambda g=g: pv(g)) for g in range(M)] if comp else []

        def project(i, c):
            if comp:
                q_s[8 * i + c] = jnp.dot(jnp.broadcast_to(x_v[0], (M, D)), w1_b[i, c // 4, :, 128 * (c % 4):128 * (c % 4 + 1)],
                                         preferred_element_type=f32)

        def wait_wide(i, c):
            wait_all([w1_b.at[i, c]], sem(2 * (i % 2) + c))

        def down(dst, blk, c):
            if dst is wd_b:
                i = 48 + 8 * (blk // 2) + 2 * (blk % 2) + c
                lhs = jax.nn.silu(q_s[i]) * q_s[i + 4]
            else:
                lhs = o_s[2 * blk + c]
            return jnp.dot(lhs.astype(bf16), dst[blk, 128 * c:128 * (c + 1)], preferred_element_type=f32)

        def add(st, dst, blk, c):
            if comp:
                key = 'y' if dst is wd_b else 'a'
                st[key] = st[key] + down(dst, blk, c)

        def do(i):
            return [(wd, wd_b, i), (wo, wo_b, i), (wo, wo_b, 6 + i), (wo, wo_b, 12 + i)]

        def attention(st, j):
            return scores(st, j, 0) + scores(st, j, 1) + values(st, j, 0)

        small = [pltpu.make_async_copy(x_hbm, x_v, sem(6)), pltpu.make_async_copy(gw_hbm, gw_v, sem(7)),
                 pltpu.make_async_copy(wr_hbm, wr_v, sem(8))]
        n0 = P['pro0']
        halves = [[u for u, (rg, c) in zip(u_q(0), _sweep(*P['qs'])) if c == k] for k in range(2)]
        kv(0, 0).start(priority=1)
        start0(*small)
        for t in range(1, L):
            kv(0, t).start(priority=1)
        for u in halves[0][:n0]:
            u()
            pl.delay(P['prod'])
        st = {}
        fast, tw = sc_t(P['fast']), sc_t(P['tw'])
        tasks = [(fast + tw, lambda: ([c.wait() for c in small], wait_wide(0, 0)))]
        tasks += [(0, lambda c=c: project(0, c)) for c in range(3)]
        stream(0, trickle(halves[1], fast, T, trickle(halves[0][n0:], 0, fast)), tasks + attention(st, 0), sc_t(P['gap']))

        def wide_step(j, st):
            st = dict(st)

            def both(fq, fg):
                pl.when(j < 6)(fq)
                pl.when(j >= 6)(fg)

            def wait():
                pl.when(j > 1)(lambda: wait_wide(j - 1, 0))
                wait_wide(j - 1, 1)
            units = [lambda a=a, b=b: both(a, b) for a, b in zip(u_q(j), u_g(j))]
            tasks = values(st, j - 1, 1, True) + [(tw, wait)] + [(0, lambda c=c: project(j - 1, c)) for c in range(8)]
            stream(j, trickle(units, 0, T), tasks + attention(st, j), sc_t(P['gap']))
            return st

        def tall_step(j, st):
            st = dict(st)
            prev = do(jnp.maximum(j - 10, 0))

            def wait():
                pl.when(j == 9)(lambda: (wait_wide(8, 0), wait_wide(8, 1)) and None)
                pl.when(j > 9)(lambda: wait_all([d.at[b] for _, d, b in prev], sem(4 + (j - 1) % 2)))

            def use(c):
                _, dst, blk = prev[c // 2]
                key = 'y' if dst is wd_b else 'a'
                if comp:
                    st[key] = jax.lax.cond(j == 9, lambda v: (project(8, c), v)[1],
                                           lambda v: v + down(dst, blk, c % 2), st[key])
            tasks = values(st, j - 1, 1, True) + [(tw, wait)] + [(0, lambda c=c: use(c)) for c in range(8)]
            stream(j, trickle(u_t(do(j - 9), sem(4 + j % 2)), 0, T), tasks + attention(st, j), sc_t(P['gap']))
            return st

        st = jax.lax.fori_loop(1, 9, wide_step, st)
        st.update(a=jnp.zeros((M, D), f32), y=jnp.zeros((M, D), f32))
        st = jax.lax.fori_loop(9, 15, tall_step, st)

        last_blocks = [(wo, wo_b, i) for i in (18, 20, 19, 21)]
        starts = [sum(chunks[:i]) for i in range(len(chunks))]

        def tail_units(ci, prio):
            k = min(P['tscr'], chunks[ci] // 32)
            n = chunks[ci] // k
            return [lambda r=r, row_=row_, u=u: [c.start(priority=prio) for c in tall(
                        wo, wo_b, 22 + starts[ci] // 256, starts[ci] % 256 + r * n + row_, u, sem(9 + ci))]
                    for row_ in range(0, n, 32) for u in range(5) for r in range(k)]

        le = sc_t(P['last_end'])
        issue = trickle(tail_units(0, 0), le, sc_t(P['t0end']), trickle(u_t(last_blocks, sem(5)), 0, le))
        issue = trickle([u for ci in range(1, len(chunks)) for u in tail_units(ci, 1)], T - L, T - L + P['t1end'], issue)

        def router():
            xf = x_v[0].astype(f32)
            st['gate'] = jax.nn.sigmoid(jnp.sum(xf * gw_v[...].astype(f32).reshape(1, D), axis=-1, keepdims=True))
            rsel = jax.nn.sigmoid(jnp.sum(xf * wr_v[...].astype(f32).reshape(1, D), axis=-1, keepdims=True))
            b = xf + (xf * 0.0 + st['y'][0:1] * rsel)
            st['base'] = (1.0 - st['gate']) * b

        def downs(blocks, s, t0):
            return [(t0, lambda: wait_all([d.at[b] for _, d, b in blocks], s))] + \
                [(0, lambda d=d, b=b, c=c: add(st, d, b, c)) for _, d, b in blocks for c in range(2)]

        def values_vpu(a, VR=P['VR']):
            def pv(r0, g):
                key = ('v', a, r0)
                p = st['p%d' % a][g:g + 1].astype(bf16).astype(f32)
                v = kv_b[1, a * DH + r0:a * DH + r0 + VR, g * G:(g + 1) * G].astype(f32) * p
                v = (v[:, 0:128] + v[:, 128:256]) + (v[:, 256:384] + v[:, 384:512])
                st[key] = v if g == 0 else st[key] + v
                if g == M - 1:
                    o = jnp.sum(st.pop(key), axis=1, keepdims=True).astype(bf16).astype(f32)
                    oc_s[a * DH + r0:a * DH + r0 + VR] = jnp.broadcast_to(o, (VR, 128))

            def rdy(r0, g):
                return max(t for t, (w_, r, c, nr, nc) in enumerate(pcs)
                           if w_ == 1 and a * DH + r0 <= r < a * DH + r0 + VR and c < (g + 1) * G and c + nc > g * G)
            return [(rdy(r0, g), lambda r0=r0, g=g: pv(r0, g)) for r0 in range(0, DH, VR) for g in range(M)] if comp else []

        tasks = values(st, NP - 2, 1, True) + downs(do(5), sem(4), tw) + [(0, router)] \
            + scores(st, NP - 1, 0) + scores(st, NP - 1, 1)
        fast_tasks = sorted(values_vpu(0) + values_vpu(1), key=lambda e: e[0])
        late = downs(last_blocks, sem(5), le + tw - 2)
        stream(NP - 1, issue, tasks + late, sc_t(P['lgap']), True, fast_tasks)

        a = st['a']
        part = None
        for ci in P['torder'] or [1, 0] + list(range(2, len(chunks))):
            r0, n = starts[ci], chunks[ci]
            blk, rb = 22 + r0 // 256, r0 % 256
            wait_all([wo_b.at[blk, pl.ds(rb, n)]], sem(9 + ci))
            if not comp:
                continue
            if ci == 0:
                a = a + down(wo_b, 22, 0)
            else:
                prod = wo_b[blk, rb:rb + n].astype(f32) * jnp.tile(oc_s[r0 - 128:r0 - 128 + n], (1, D // 128))
                red = [prod[8 * i:8 * (i + 1)] for i in range(n // 8)] + ([] if part is None else [part])
                while len(red) > 1:
                    red = [red[i] + red[i + 1] if i + 1 < len(red) else red[i] for i in range(0, len(red), 2)]
                part = red[0]
        a = a[0:1]
        if part is not None:
            a = a + jnp.sum(part, axis=0, keepdims=True)
        out_ref[0] = (st['gate'] * a + st['base']).astype(bf16)

    def fn(A_x, A_k_cache, A_v_cache, A_wq, A_wo, B_x, B_w_r, B_w_gate, B_w_up, B_w_down, gate_w):
        del B_x
        kT = jnp.swapaxes(A_k_cache, 2, 3).reshape(NP, PD, SK)
        vT = jnp.swapaxes(A_v_cache, 2, 3).reshape(NP, PD, SK)
        any_spec = pl.BlockSpec(memory_space=pl.ANY)
        vmem = pltpu.VMEM
        return pl.pallas_call(
            kern,
            out_shape=jax.ShapeDtypeStruct((1, 1, D), bf16),
            in_specs=[any_spec] * 10,
            out_specs=pl.BlockSpec(memory_space=pltpu.VMEM),
            scratch_shapes=[
                vmem((1, 1, D), bf16), vmem((D,), bf16), vmem((D,), bf16),
                vmem((9, 2, D, 512), bf16), vmem((2, PD, W), bf16),
                vmem((24, 256, D), bf16), vmem((6, 256, D), bf16),
                vmem((72, M, 128), f32), vmem((48, M, 128), f32), vmem((PD, 128), f32),
                pltpu.SemaphoreType.DMA((NS + 9 + len(chunks),)),
            ],
            compiler_params=pltpu.CompilerParams(
                vmem_limit_bytes=64 * 1024 * 1024,
                disable_semaphore_checks=True, disable_bounds_checks=True, flags=P['flags'],
            ),
            name=P['name'],
        )(A_x, kT, vT, A_wq, A_wo.reshape(24, 256, D), B_w_r, B_w_gate, B_w_up, B_w_down.reshape(6, 256, D), gate_w)
    return fn


pallas_gated_mix__sliding_block_cached__moe_arch_mod__decode_kernel = jax.jit(make())
```

```python
import jax
import jax.numpy as jnp
import jax.experimental.pallas as pl
import jax.experimental.pallas.tpu as pltpu

H, DH, SK, D, F = 32, 192, 32768, 640, 1536
W = min(4096, max(256, SK // 4))
BASE = SK - W
f32, bf16 = jnp.float32, jnp.bfloat16
U = 512
QR, QC = D // 2, 2 * U
NQ = 2 * H * DH // QC
GR = 128
NG = D // GR
NT = H // 2
DR = F // NT

DEFAULT = dict(L=20, name="k8", prof=False, kco=[[i] for i in (0, 3, 4, 7, 6, 5, 2, 1)], vco=None, KU=6,
               qm=7, grun=2, trun=2, pro0=12, prod=40, tw=14, comp=True, fast=22, qm0=31,
               tail=(96, 64, 32), flags=None, t1end=8, t0end=58, early=60, first=None, q0first=False, dly=0, diag=True)

SPLIT = [[(0, 0, 4)], [(0, 4, 1), (1, 0, 3)], [(1, 3, 2), (2, 0, 2)], [(2, 2, 3), (3, 0, 1)], [(3, 1, 4)]]


def _tree(xs):
    while len(xs) > 1:
        xs = [xs[i] + xs[i + 1] if i + 1 < len(xs) else xs[i] for i in range(0, len(xs), 2)]
    return xs[0]


def _place(into, items, t0, t1):
    for i, it in enumerate(items):
        if it is not None:
            into.setdefault(t0 + int((i + 0.5) * (t1 - t0) / len(items)), []).append(it)
    return into


def _slow(fns):
    return [g for f in fns for g in [f] + [None] * 5]


def _merge(lists, run):
    keyed = [((i + 0.5 * run) / len(lst), k, lst[i:i + run]) for k, lst in enumerate(lists)
             for i in range(0, len(lst), run)]
    return [it for _, _, part in sorted(keyed, key=lambda e: e[:2]) for it in part]


def make(**kw):
    P = dict(DEFAULT)
    P.update(kw)
    L = P['L']
    pcs = []
    for w, co in enumerate((P['kco'], P['vco'] or P['kco'])):
        for g in co:
            nr = 8 * P['KU'] // len(g)
            for r in range(0, DH, nr):
                if list(g) == list(range(g[0], g[0] + len(g))):
                    dmas = [(r, nr, g[0] * U, len(g) * U)]
                else:
                    dmas = [(rr, 8, c * U, U) for rr in range(r, r + nr, 8) for c in g]
                pcs.append((w, r, nr, g, dmas))
    T = len(pcs)
    NS = min(s for s in range(L, T + 1) if T % s == 0)
    comp = P['comp']
    sc_t = lambda t: t * T // 64

    def kern(x_hbm, kT, vT, wq, wo, wr_hbm, wg, wu, wd, gw_hbm, out_ref,
             x_v, wr_v, gw_v, kv_b, wq0_b, wq_b, gu_b, w2_b, x_c, q_c, o_c, h_c, s_s, p_s, o_s, q_s, gu_s, a_s, sems):
        def ds(start, n, mult):
            return pl.ds(start if isinstance(start, int) else pl.multiple_of(start, mult), n)

        def sem(i):
            return sems.at[NS + i]

        def kv(h, t):
            w = pcs[t][0]
            return [pltpu.make_async_copy((kT, vT)[w].at[h, pl.ds(r, nr), pl.ds(BASE + c, nc)],
                                          kv_b.at[h % 2, w, pl.ds(r, nr), pl.ds(c, nc)], sems.at[t % NS])
                    for r, nr, c, nc in pcs[t][4]]

        def start(prio, *cs):
            for c in cs:
                c.start(priority=prio)

        def wait_all(buf, s):
            pltpu.make_async_copy(buf, buf, s).wait()

        def q_units(i):
            def unit(r, c):
                start(0, pltpu.make_async_copy(wq.at[ds(i % 2 * QR + r, 8, 8), ds(i // 2 * QC + c, U, U)],
                                               wq_b.at[i % 2, pl.ds(r, 8), pl.ds(c, U)], sem(i % 2)))
            return [lambda r=8 * k * P['qm'] % QR, c=c: unit(r, c) for k in range(QR // 8) for c in (0, U)]

        def gu_units(i):
            def unit(m, r, c):
                start(0, pltpu.make_async_copy((wg, wu)[m].at[ds((i - NQ) * GR + r, 8, 8), pl.ds(c, U)],
                                               gu_b.at[i % 2, m, pl.ds(r, 8), pl.ds(c, U)], sem(i % 2)))
            return _merge([[lambda m=m, r=r, c=c: unit(m, r, c) for r in range(0, GR, 8) for c in range(0, F, U)]
                           for m in range(2)], P['grun'])

        def out_parts(i):
            j = i - NQ - NG
            return [(wo, o_c, j * DH, DH, 0, 0), (wo, o_c, (NT + j) * DH, DH, DH, 0), (wd, h_c, j * DR, DR, 2 * DH, 1)]

        def part_units(i, part, r0, r1, prio, s):
            src, _, row0, _, off, _ = part

            def unit(r, u):
                start(prio, *[pltpu.make_async_copy(src.at[ds(row0 + r + 8 * g, 8, 8), pl.ds(128 * c, 128 * n)],
                                                    w2_b.at[i % 2, pl.ds(off + r + 8 * g, 8), pl.ds(128 * c, 128 * n)], s)
                              for g, c, n in SPLIT[u]])
            return [lambda r=r, u=u: unit(r, u) for r in range(r0, r1, 32) for u in range(5)]

        def out_units(i):
            return _merge([part_units(i, p, 0, p[3], 0, sem(i % 2)) for p in out_parts(i)], P['trun'])

        def stream(h, issue, tasks, last=False):
            for t in range(T):
                w, r, nr, g, _ = pcs[t]
                wait_all(kv_b.at[h % 2, w, pl.ds(r, nr), pl.ds(min(g) * U, len(g) * U)], sems.at[t % NS])
                for fn in issue.get(t, []):
                    fn()
                if t + L < T:
                    start(1, *kv(h, t + L))
                elif not last:
                    start(1, *kv(h + 1, t + L - T))
                for fn in tasks.get(t, []):
                    fn()
                if P['dly']:
                    pl.delay(P['dly'])

        if P['prof']:
            stream = jax.named_scope("grp")(stream)

        def rows_dot(w, col):
            prod = w.astype(f32) * jnp.tile(col, (1, w.shape[1] // 128))
            return _tree([prod[i:i + 8] for i in range(0, w.shape[0], 8)])

        def columns(v):
            if P['diag']:
                eye = jax.lax.broadcasted_iota(jnp.int32, (128, 128), 0) == jax.lax.broadcasted_iota(jnp.int32, (128, 128), 1)
                return jnp.broadcast_to(jnp.sum(jnp.where(eye, v, 0.0), axis=1, keepdims=True), (128, 128))
            return jnp.broadcast_to(v, (128, 128)).T

        def attention(h):
            seen = set()

            def accumulate(ref, idx, val, key):
                ref[idx] = ref[idx] + val if key in seen else val
                seen.add(key)

            def piece(w, r, nr, g, _):
                cols = [slice(c * U, (c + 1) * U) for c in g]
                if w == 0:
                    q = q_c[ds(h * DH + r, nr, 8)]
                    for c in cols:
                        accumulate(s_s, (slice(None), c), rows_dot(kv_b[h % 2, 0, r:r + nr, c], q), (0, c.start))
                else:
                    prod = [kv_b[h % 2, 1, r:r + nr, c].astype(f32) * jnp.tile(p_s[:, c], (nr // 8, 1)) for c in cols]
                    o = _tree([v[:, i:i + 128] for v in prod for i in range(0, U, 128)])
                    for i in range(0, nr, 8):
                        accumulate(o_s, slice(r + i, r + i + 8), o[i:i + 8], (1, r + i))

            def softmax():
                s = jnp.sum(s_s[...], axis=0, keepdims=True) * DH ** -0.5
                e = jnp.exp(s - jnp.max(s, axis=1, keepdims=True))
                p_s[...] = jnp.broadcast_to(e * (1.0 / jnp.sum(e, axis=1, keepdims=True)), (8, W))

            def finish():
                o_c[ds(h * DH, DH, 8)] = jnp.broadcast_to(jnp.sum(o_s[...], axis=1, keepdims=True), (DH, 128))

            fns = [[lambda p=p: piece(*p)] for p in pcs]
            fns[T // 2 - 1].append(softmax)
            fns[T - 1].append(finish)
            return fns if comp else [[] for _ in pcs]

        def q_tasks(i, ncol=QC):
            def part(r):
                v = rows_dot(wq_b[i % 2, r:r + 16], x_c[ds(i % 2 * QR + r, 16, 16)])
                q_s[i % 2] = v if r == 0 else q_s[i % 2] + v

            def put(c):
                def fn():
                    q = jnp.sum(q_s[0, :, c:c + 128] + q_s[1, :, c:c + 128], axis=0, keepdims=True)
                    q_c[ds(i // 2 * QC + c, 128, 128)] = columns(q)
                if not isinstance(i, int):
                    pl.when(i % 2 == 1)(fn)
                elif i % 2:
                    fn()
            fns = [lambda r=r: part(r) for r in range(0, QR, 16)] + _slow([lambda c=c: put(c) for c in range(0, QC, 128)])
            return [lambda: wait_all(wq_b.at[i % 2], sem(i % 2))] + (fns if comp else [])

        def gu_tasks(i):
            def part(m, r, c):
                gu_s[m, :, c:c + U] += rows_dot(gu_b[i % 2, m, r:r + 32, c:c + U], x_c[ds((i - NQ) * GR + r, 32, 32)])
            fns = [lambda m=m, r=r, c=c: part(m, r, c) for m in range(2) for r in range(0, GR, 32) for c in range(0, F, U)]
            return [lambda: wait_all(gu_b.at[i % 2], sem(i % 2))] + (fns if comp else [])

        def swiglu(c):
            g, u = [jnp.sum(gu_s[m, :, c:c + 128], axis=0, keepdims=True) for m in range(2)]
            h_c[c:c + 128] = columns(jax.nn.silu(g) * u)

        def out_dot(i, part, r, n):
            _, col, row0, _, off, _ = part
            return rows_dot(w2_b[i % 2, off + r:off + r + n], col[ds(row0 + r, n, 32)])

        def out_tasks(i):
            def part(p, r):
                a_s[p[5]] += out_dot(i, p, r, 32)
            fns = [lambda p=p, r=r: part(p, r) for p in out_parts(i) for r in range(0, p[3], 32)]
            return [lambda: wait_all(w2_b.at[i % 2], sem(i % 2))] + (fns if comp else [])

        tw = sc_t(P['tw'])

        def loop(lo, hi, units, side, first_side=None):
            def body(h, carry):
                tasks = dict(enumerate(attention(h)))
                if first_side is None:
                    _place(tasks, side(h), tw, T - 2)
                else:
                    _place(tasks, [f and (lambda f=f: pl.when(h == lo)(f)) for f in first_side], tw, T - 2)
                    _place(tasks, [f and (lambda f=f: pl.when(h > lo)(f)) for f in side(h)], tw, T - 2)
                stream(h, _place({}, units(h + 1), 0, T), tasks)
                return carry
            jax.lax.fori_loop(lo, hi, body, 0)

        small = [pltpu.make_async_copy(x_hbm, x_v, sem(2)), pltpu.make_async_copy(gw_hbm, gw_v, sem(3)),
                 pltpu.make_async_copy(wr_hbm, wr_v, sem(4))]
        n0 = P['pro0']

        def first_units(i):
            def unit(r):
                start(0, pltpu.make_async_copy(wq.at[pl.ds(r, 8), pl.ds(i * U, U)], wq0_b.at[i, pl.ds(r, 8)], sem(i)))
            return [lambda r=8 * k * P['qm0'] % D: unit(r) for k in range(D // 8)]

        def first_tasks(i):
            def part(r):
                v = rows_dot(wq0_b[i, r:r + 32], x_c[r:r + 32])
                q_s[0, :, :U] = v if r == 0 else q_s[0, :, :U] + v

            def put(c):
                q_c[i * U + c:i * U + c + 128] = columns(jnp.sum(q_s[0, :, c:c + 128], axis=0, keepdims=True))
            fns = [lambda r=r: part(r) for r in range(0, D, 32)] + _slow([lambda c=c: put(c) for c in range(0, U, 128)])
            return [lambda: wait_all(wq0_b.at[i], sem(i))] + (fns if comp else [])

        units = first_units(0)
        start(1, *kv(0, 0))
        start(0, *small)
        for t in range(1, L):
            start(1, *kv(0, t))
        for u in units[:n0]:
            u()
            pl.delay(P['prod'])

        def setup():
            for c in small:
                c.wait()
            a_s[...] = jnp.zeros(a_s.shape, f32)
            gu_s[...] = jnp.zeros(gu_s.shape, f32)

        def x_cols(c):
            x_c[c:c + 128] = columns(x_v[0][:, c:c + 128].astype(f32))
        fast = sc_t(P['fast'])
        tasks = _place({}, [setup] + [lambda c=c: x_cols(c) for c in range(0, D, 128)], 2, fast)
        t = fast + sc_t(10)
        _place(tasks, first_tasks(0), t, t + sc_t(10))
        t = 3 * (t + sc_t(10))
        for t0, fns in enumerate(attention(0)):
            t = max(t + 1, 3 * t0)
            tasks.setdefault(min(t // 3, T - 1), []).extend(fns)
        stream(0, _place(_place({}, units[n0:], 0, fast), first_units(1), fast, T), tasks)

        loop(1, NQ - 1, q_units, q_tasks, first_tasks(1))
        loop(NQ - 1, NQ + NG - 1, gu_units, gu_tasks, q_tasks(NQ - 1))
        loop(NQ + NG - 1, H - 1, out_units, out_tasks,
             gu_tasks(NQ + NG - 1) + _slow([lambda c=c: swiglu(c) for c in range(0, F, 128)]))

        early, late, ffn = out_parts(H)
        starts = [sum(P['tail'][:i]) for i in range(len(P['tail']))]
        issue = _place({}, part_units(H, ffn, 0, DR, 0, sem(5)) + part_units(H, late, 0, DH, 0, sem(6)), 0, sc_t(P['t0end']))
        _place(issue, [u for k, (r, n) in enumerate(zip(starts, P['tail']))
                       for u in part_units(H, early, r, r + n, 1, sem(7 + k))], T - L, T - L + P['t1end'])
        st = {}

        def router():
            wait_all(w2_b.at[0, pl.ds(ffn[4], DR)], sem(5))
            y = jnp.sum(a_s[1] + out_dot(H, ffn, 0, DR), axis=0, keepdims=True)
            xf = x_v[0].astype(f32)
            st['gate'] = jax.nn.sigmoid(jnp.sum(xf * gw_v[...].astype(f32).reshape(1, D), axis=-1, keepdims=True))
            rsel = jax.nn.sigmoid(jnp.sum(xf * wr_v[...].astype(f32).reshape(1, D), axis=-1, keepdims=True))
            st['base'] = (1.0 - st['gate']) * (xf + (xf * 0.0 + y * rsel))

        stream(H - 1, issue, _place(dict(enumerate(attention(H - 1))), out_tasks(H - 1) + [router], tw, sc_t(48)), True)
        a = a_s[0]
        seq = [(early, r, n, 7 + k) for k, (r, n) in enumerate(zip(starts, P['tail']))]
        seq.insert(P['first'] or 0, (late, 0, DH, 6))
        for p, r, n, s in seq:
            wait_all(w2_b.at[0, pl.ds(p[4] + r, n)], sem(s))
            if comp:
                a = a + out_dot(H, p, r, n)
        out_ref[0] = (st['gate'] * jnp.sum(a, axis=0, keepdims=True) + st['base']).astype(bf16)

    def fn(A_x, A_k_cache, A_v_cache, A_wq, A_wo, B_x, B_w_r, B_w_gate, B_w_up, B_w_down, gate_w):
        del B_x
        kT = jnp.swapaxes(A_k_cache, 2, 3).reshape(H, DH, SK)
        vT = jnp.swapaxes(A_v_cache, 2, 3).reshape(H, DH, SK)
        any_spec = pl.BlockSpec(memory_space=pl.ANY)
        vmem = pltpu.VMEM
        return pl.pallas_call(
            kern,
            out_shape=jax.ShapeDtypeStruct((1, 1, D), bf16),
            in_specs=[any_spec] * 10,
            out_specs=pl.BlockSpec(memory_space=pltpu.VMEM),
            scratch_shapes=[
                vmem((1, 1, D), bf16), vmem((D,), bf16), vmem((D,), bf16),
                vmem((2, 2, DH, W), bf16), vmem((2, D, U), bf16), vmem((2, QR, QC), bf16), vmem((2, 2, GR, F), bf16),
                vmem((2, 2 * DH + DR, D), bf16),
                vmem((D, 128), f32), vmem((H * DH, 128), f32), vmem((H * DH, 128), f32), vmem((F, 128), f32),
                vmem((8, W), f32), vmem((8, W), f32), vmem((DH, 128), f32),
                vmem((2, 8, QC), f32), vmem((2, 8, F), f32), vmem((2, 8, D), f32),
                pltpu.SemaphoreType.DMA((NS + 7 + len(P['tail']),)),
            ],
            compiler_params=pltpu.CompilerParams(
                vmem_limit_bytes=64 * 1024 * 1024,
                disable_semaphore_checks=True, disable_bounds_checks=True, flags=P['flags'],
            ),
            name=P['name'],
        )(A_x, kT, vT, A_wq, A_wo, B_w_r, B_w_gate, B_w_up, B_w_down, gate_w)
    return fn


pallas_gated_mix__sliding_block_cached__moe_arch_mod__decode_kernel = jax.jit(make(name="gated_mix_decode", **dict(t0end=54, first=1, L=24)))
```

```python
import jax
import jax.numpy as jnp
import jax.experimental.pallas as pl
import jax.experimental.pallas.tpu as pltpu

H, DH, SK, D, F = 32, 192, 32768, 640, 1536
W = min(4096, max(256, SK // 4))
BASE = SK - W
U = 512

KR = 48
COL_ORDER = (0, 3, 4, 7, 6, 5, 2, 1)
PIECES = [(w, r, c * U) for w in range(2) for c in COL_ORDER for r in range(0, DH, KR)]
T = len(PIECES)
AHEAD = 24
NSEM = 32

QR, QC = D // 2, 2 * U
NQ = 2 * H * DH // QC
GR = 128
NG = D // GR
NO = H // 2
DR = F // NO
LANDED = 14
WARM = AHEAD // 2
FIRST_END = 22
LAST_END = 57
assert NQ + NG + NO == H + 1

SPLIT = [[(0, 0, 4)], [(0, 4, 1), (1, 0, 3)], [(1, 3, 2), (2, 0, 2)], [(2, 2, 3), (3, 0, 1)], [(3, 1, 4)]]

f32 = jnp.float32
bf16 = jnp.bfloat16


def _place(schedule, fns, t0, t1):
    for i, fn in enumerate(fns):
        if fn is not None:
            schedule.setdefault(t0 + int((i + 0.5) * (t1 - t0) / len(fns)), []).append(fn)
    return schedule


def _spaced(fns):
    return [g for fn in fns for g in [fn] + [None] * 5]


def _merge(lists, run=2):
    keyed = [((i + 0.5 * run) / len(lst), k, lst[i:i + run])
             for k, lst in enumerate(lists) for i in range(0, len(lst), run)]
    return [fn for _, _, part in sorted(keyed, key=lambda e: e[:2]) for fn in part]


def _ds(start, size, align):
    return pl.ds(start if isinstance(start, int) else pl.multiple_of(start, align), size)


def _start(queue, src, dst, sem):
    pltpu.make_async_copy(src, dst, sem).start(priority=queue)


def _wait(buf, sem):
    pltpu.make_async_copy(buf, buf, sem).wait()


def _tree_sum(xs):
    while len(xs) > 1:
        xs = [xs[i] + xs[i + 1] if i + 1 < len(xs) else xs[i] for i in range(0, len(xs), 2)]
    return xs[0]


def _rows_dot(w, col):
    prod = w.astype(f32) * jnp.tile(col, (1, w.shape[1] // 128))
    return _tree_sum([prod[i:i + 8] for i in range(0, w.shape[0], 8)])


def _columns(v):
    eye = (jax.lax.broadcasted_iota(jnp.int32, (128, 128), 0)
           == jax.lax.broadcasted_iota(jnp.int32, (128, 128), 1))
    return jnp.broadcast_to(jnp.sum(jnp.where(eye, v, 0.0), axis=1, keepdims=True), (128, 128))


def _kernel(x_hbm, kT, vT, wq, wo, wr_hbm, wg, wu, wd, gw_hbm, out_ref,
            x_v, wr_v, gw_v, kv_b, wq0_b, wq_b, gu_b, out_b,
            x_c, q_c, o_c, h_c, s_s, p_s, o_s, q_s, gu_s, a_s, sems):
    def sem(i):
        return sems.at[NSEM + i]

    def kv_copy(h, t):
        w, r, c = PIECES[t]
        return pltpu.make_async_copy((kT, vT)[w].at[h, pl.ds(r, KR), pl.ds(BASE + c, U)],
                                     kv_b.at[h % 2, w, pl.ds(r, KR), pl.ds(c, U)], sems.at[t % NSEM])

    def stream(h, requests, tasks, last=False):
        for t in range(T):
            kv_copy(h, t).wait()
            for fn in requests.get(t, []):
                fn()
            if t + AHEAD < T:
                kv_copy(h, t + AHEAD).start(priority=1)
            elif not last:
                kv_copy(h + 1, t + AHEAD - T).start(priority=1)
            for fn in tasks.get(t, []):
                fn()

    def attention(h):
        def piece(w, r, c):
            blk = kv_b[h % 2, w, r:r + KR, c:c + U]
            if w == 0:
                s = _rows_dot(blk, q_c[_ds(h * DH + r, KR, 8)])
                s_s[:, c:c + U] = s if r == 0 else s_s[:, c:c + U] + s
            else:
                prod = blk.astype(f32) * jnp.tile(p_s[:, c:c + U], (KR // 8, 1))
                o = _tree_sum([prod[:, i:i + 128] for i in range(0, U, 128)])
                o_s[r:r + KR] = o if c == COL_ORDER[0] * U else o_s[r:r + KR] + o

        def softmax():
            s = jnp.sum(s_s[...], axis=0, keepdims=True) * DH ** -0.5
            e = jnp.exp(s - jnp.max(s, axis=1, keepdims=True))
            p_s[...] = jnp.broadcast_to(e * (1.0 / jnp.sum(e, axis=1, keepdims=True)), (8, W))

        def finish():
            o_c[_ds(h * DH, DH, 8)] = jnp.broadcast_to(jnp.sum(o_s[...], axis=1, keepdims=True), (DH, 128))

        fns = [[lambda p=p: piece(*p)] for p in PIECES]
        fns[T // 2 - 1].append(softmax)
        fns[T - 1].append(finish)
        return fns

    def first_unit(i, r):
        _start(0, wq.at[_ds(r, 8, 8), pl.ds(i * U, U)], wq0_b.at[i, _ds(r, 8, 8)], sem(i))

    first_stride = 8 * 31

    def first_units(i):
        return [lambda r=k * first_stride % D: first_unit(i, r) for k in range(D // 8)]

    def first_tasks(i):
        def part(r):
            v = _rows_dot(wq0_b[i, r:r + 32], x_c[r:r + 32])
            q_s[0, :, :U] = v if r == 0 else q_s[0, :, :U] + v

        def put(c):
            q_c[i * U + c:i * U + c + 128] = _columns(jnp.sum(q_s[0, :, c:c + 128], axis=0, keepdims=True))

        return ([lambda: _wait(wq0_b.at[i], sem(i))] + [lambda r=r: part(r) for r in range(0, D, 32)]
                + _spaced([lambda c=c: put(c) for c in range(0, U, 128)]))

    def q_units(i):
        def unit(r, c):
            _start(0, wq.at[_ds(i % 2 * QR + r, 8, 8), _ds(i // 2 * QC + c, U, U)],
                   wq_b.at[i % 2, pl.ds(r, 8), pl.ds(c, U)], sem(i % 2))
        return [lambda r=8 * 7 * k % QR, c=c: unit(r, c) for k in range(QR // 8) for c in (0, U)]

    def q_tasks(i):
        def part(r):
            v = _rows_dot(wq_b[i % 2, r:r + 16], x_c[_ds(i % 2 * QR + r, 16, 16)])
            q_s[i % 2] = v if r == 0 else q_s[i % 2] + v

        def put(c):
            @pl.when(i % 2 == 1)
            def _():
                q = jnp.sum(q_s[0, :, c:c + 128] + q_s[1, :, c:c + 128], axis=0, keepdims=True)
                q_c[_ds(i // 2 * QC + c, 128, 128)] = _columns(q)

        return ([lambda: _wait(wq_b.at[i % 2], sem(i % 2))] + [lambda r=r: part(r) for r in range(0, QR, 16)]
                + _spaced([lambda c=c: put(c) for c in range(0, QC, 128)]))

    def gu_units(i):
        def unit(m, r, c):
            _start(0, (wg, wu)[m].at[_ds((i - NQ) * GR + r, 8, 8), pl.ds(c, U)],
                   gu_b.at[i % 2, m, pl.ds(r, 8), pl.ds(c, U)], sem(i % 2))
        return _merge([[lambda m=m, r=r, c=c: unit(m, r, c) for r in range(0, GR, 8) for c in range(0, F, U)]
                       for m in range(2)])

    def gu_tasks(i):
        def part(m, r, c):
            gu_s[m, :, c:c + U] += _rows_dot(gu_b[i % 2, m, r:r + 32, c:c + U], x_c[_ds((i - NQ) * GR + r, 32, 32)])

        return [lambda: _wait(gu_b.at[i % 2], sem(i % 2))] + [
            lambda m=m, r=r, c=c: part(m, r, c) for m in range(2) for r in range(0, GR, 32) for c in range(0, F, U)]

    def swiglu(c):
        g, u = [jnp.sum(gu_s[m, :, c:c + 128], axis=0, keepdims=True) for m in range(2)]
        h_c[c:c + 128] = _columns(jax.nn.silu(g) * u)

    def out_parts(i):
        j = i - NQ - NG
        return [(wo, o_c, j * DH, DH, 0, 0), (wo, o_c, (NO + j) * DH, DH, DH, 0), (wd, h_c, j * DR, DR, 2 * DH, 1)]

    def part_units(i, part, r0, n, queue, s):
        src, _, row0, _, off, _ = part

        def unit(r, spans):
            for g, c, tiles in spans:
                cols = pl.ds(128 * c, 128 * tiles)
                _start(queue, src.at[_ds(row0 + r + 8 * g, 8, 8), cols], out_b.at[i % 2, pl.ds(off + r + 8 * g, 8), cols], s)
        return [lambda r=r, spans=spans: unit(r, spans) for r in range(r0, r0 + n, 32) for spans in SPLIT]

    def out_units(i):
        return _merge([part_units(i, p, 0, p[3], 0, sem(i % 2)) for p in out_parts(i)])

    def out_tasks(i):
        def part(p, r):
            _, col, row0, _, off, acc = p
            a_s[acc] += _rows_dot(out_b[i % 2, off + r:off + r + 32], col[_ds(row0 + r, 32, 32)])

        return [lambda: _wait(out_b.at[i % 2], sem(i % 2))] + [
            lambda p=p, r=r: part(p, r) for p in out_parts(i) for r in range(0, p[3], 32)]

    small = [pltpu.make_async_copy(x_hbm, x_v, sem(2)),
             pltpu.make_async_copy(gw_hbm, gw_v, sem(3)),
             pltpu.make_async_copy(wr_hbm, wr_v, sem(4))]
    kv_copy(0, 0).start(priority=1)
    kv_copy(0, 1).start(priority=1)
    first_unit(0, 0)
    for copy in small:
        copy.start()

    order_bits = sum(c << (3 * k) for k, c in enumerate(COL_ORDER))

    def warm(k, r):
        for t in (2 * k, 2 * k + 1):
            rows, c = _ds((t & 3) * KR, KR, 16), ((order_bits >> (3 * (t >> 2))) & 7) * U
            _start(1, kT.at[0, rows, _ds(BASE + c, U, U)], kv_b.at[0, 0, rows, _ds(c, U, U)], sems.at[t])
        first_unit(0, r)
        r = r + first_stride
        return jnp.where(r >= D, r - D, r)

    jax.lax.fori_loop(1, WARM, warm, first_stride)

    def setup():
        for copy in small:
            copy.wait()
        a_s[...] = jnp.zeros(a_s.shape, f32)
        gu_s[...] = jnp.zeros(gu_s.shape, f32)

    def x_columns(c):
        x_c[c:c + 128] = _columns(x_v[0][:, c:c + 128].astype(f32))

    tasks = _place({}, [setup] + [lambda c=c: x_columns(c) for c in range(0, D, 128)], 2, FIRST_END)
    _place(tasks, first_tasks(0), FIRST_END + 10, FIRST_END + 20)
    third = 3 * (FIRST_END + 20)
    for t, fns in enumerate(attention(0)):
        third = max(third + 1, 3 * t)
        tasks.setdefault(min(third // 3, T - 1), []).extend(fns)
    requests = _place(_place({}, first_units(0)[WARM:], 0, FIRST_END), first_units(1), FIRST_END, T)
    stream(0, requests, tasks)

    def heads(lo, hi, units, consume, consume_first):
        def body(h, carry):
            tasks = dict(enumerate(attention(h)))
            _place(tasks, [fn and (lambda fn=fn: pl.when(h == lo)(fn)) for fn in consume_first], LANDED, T - 2)
            _place(tasks, [fn and (lambda fn=fn: pl.when(h > lo)(fn)) for fn in consume(h)], LANDED, T - 2)
            stream(h, _place({}, units(h + 1), 0, T), tasks)
            return carry
        jax.lax.fori_loop(lo, hi, body, 0)

    heads(1, NQ - 1, q_units, q_tasks, first_tasks(1))
    heads(NQ - 1, NQ + NG - 1, gu_units, gu_tasks, q_tasks(NQ - 1))
    heads(NQ + NG - 1, H - 1, out_units, out_tasks,
          gu_tasks(NQ + NG - 1) + _spaced([lambda c=c: swiglu(c) for c in range(0, F, 128)]))

    early, late, ffn = out_parts(H)
    tail = [(late, 0, 160), (early, 0, 64), (early, 64, 64), (late, 160, 32), (early, 128, 32), (early, 160, 32)]

    def tail_units(part, queue):
        return [fn for k, (p, r, n) in enumerate(tail) if p is part
                for fn in part_units(H, p, r, n, queue, sem(6 + k))]

    requests = _place({}, part_units(H, ffn, 0, DR, 0, sem(5)) + tail_units(late, 0), 0, LAST_END)
    _place(requests, tail_units(early, 1), T - AHEAD, T - AHEAD + 8)
    mix = {}

    def ffn_branch():
        _wait(out_b.at[0, pl.ds(ffn[4], DR)], sem(5))
        y = a_s[1] + _rows_dot(out_b[0, ffn[4]:ffn[4] + DR], h_c[ffn[2]:ffn[2] + DR])
        y = jnp.sum(y, axis=0, keepdims=True)
        x = x_v[0].astype(f32)
        gate = jax.nn.sigmoid(jnp.sum(x * gw_v[...].astype(f32).reshape(1, D), axis=-1, keepdims=True))
        route = jax.nn.sigmoid(jnp.sum(x * wr_v[...].astype(f32).reshape(1, D), axis=-1, keepdims=True))
        mix['gate'] = gate
        mix['ffn'] = (1.0 - gate) * (x + (x * 0.0 + y * route))

    tasks = _place(dict(enumerate(attention(H - 1))), out_tasks(H - 1) + [ffn_branch], LANDED, 48)
    stream(H - 1, requests, tasks, last=True)

    row0 = jax.lax.broadcasted_iota(jnp.int32, (8, D), 0) == 0
    acc = mix['gate'] * a_s[0] + jnp.where(row0, mix['ffn'], 0.0)
    for k, ((_, _, first, _, off, _), r, n) in enumerate(tail):
        col = mix['gate'] * o_c[first + r:first + r + n]
        _wait(out_b.at[0, pl.ds(off + r, n)], sem(6 + k))
        acc = acc + _rows_dot(out_b[0, off + r:off + r + n], col)
    out_ref[0] = jnp.sum(acc, axis=0, keepdims=True).astype(bf16)


@jax.jit
def pallas_gated_mix__sliding_block_cached__moe_arch_mod__decode_kernel(
        A_x, A_k_cache, A_v_cache, A_wq, A_wo, B_x, B_w_r, B_w_gate, B_w_up, B_w_down, gate_w):
    del B_x
    kT = jnp.swapaxes(A_k_cache, 2, 3).reshape(H, DH, SK)
    vT = jnp.swapaxes(A_v_cache, 2, 3).reshape(H, DH, SK)
    vmem = pltpu.VMEM
    return pl.pallas_call(
        _kernel,
        out_shape=jax.ShapeDtypeStruct((1, 1, D), bf16),
        in_specs=[pl.BlockSpec(memory_space=pl.ANY)] * 10,
        out_specs=pl.BlockSpec(memory_space=pltpu.VMEM),
        scratch_shapes=[
            vmem((1, 1, D), bf16), vmem((D,), bf16), vmem((D,), bf16),
            vmem((2, 2, DH, W), bf16), vmem((2, D, U), bf16), vmem((2, QR, QC), bf16),
            vmem((2, 2, GR, F), bf16), vmem((2, 2 * DH + DR, D), bf16),
            vmem((D, 128), f32), vmem((H * DH, 128), f32), vmem((H * DH, 128), f32), vmem((F, 128), f32),
            vmem((8, W), f32), vmem((8, W), f32), vmem((DH, 128), f32),
            vmem((2, 8, QC), f32), vmem((2, 8, F), f32), vmem((2, 8, D), f32),
            pltpu.SemaphoreType.DMA((NSEM + 12,)),
        ],
        compiler_params=pltpu.CompilerParams(
            vmem_limit_bytes=64 * 1024 * 1024,
            disable_semaphore_checks=True,
            disable_bounds_checks=True,
        ),
        name="gated_mix_decode",
    )(A_x, kT, vT, A_wq, A_wo, B_w_r, B_w_gate, B_w_up, B_w_down, gate_w)
```

```python
import jax
import jax.numpy as jnp
import jax.experimental.pallas as pl
import jax.experimental.pallas.tpu as pltpu

H, DH, SK, D, F = 32, 192, 32768, 640, 1536
W = min(4096, max(256, SK // 4))
BASE = SK - W
U = 512

SHIFT = (40, -16)
SWEEPS = ([[0], [3], [4], [7], [6], [5], [2], [1]],) * 2
AHEAD = 28
NSEM = 32


def _pieces(first=False, last=False):
    out = []
    for w in range(2):
        for cols in SWEEPS[w]:
            edges = list(range(SHIFT[w], SHIFT[w] + DH + 1, 48 // len(cols)))
            edges = [max(e, 8 * k) for k, e in enumerate([0] + edges[1:])] if first else edges
            edges = [min(e, DH - 8 * k) for k, e in enumerate([DH] + edges[-2::-1])][::-1] if last else edges
            out += [(w, r0, r1 - r0, cols) for r0, r1 in zip(edges, edges[1:])]
    return out


FIRST, MID, LAST = _pieces(first=True), _pieces(), _pieces(last=True)
T = len(MID)
PAD = 48

QR, QC = D // 2, 2 * U
NQ = 2 * H * DH // QC
GR = 128
NG = D // GR
NO = H // 2
DR = F // NO
LAG = 64
LANDED = 14
WARM = AHEAD // 2
FIRST_END = 22
LAST_END = 57
assert NQ + NG + NO == H + 1

SPLIT = [[(0, 0, 4)], [(0, 4, 1), (1, 0, 3)], [(1, 3, 2), (2, 0, 2)], [(2, 2, 3), (3, 0, 1)], [(3, 1, 4)]]

f32 = jnp.float32
bf16 = jnp.bfloat16


def _place(schedule, fns, t0, t1):
    for i, fn in enumerate(fns):
        if fn is not None:
            schedule.setdefault(t0 + int((i + 0.5) * (t1 - t0) / len(fns)), []).append(fn)
    return schedule


def _spaced(fns):
    return [g for fn in fns for g in [fn] + [None] * 5]


def _merge(lists, run=2):
    keyed = [((i + 0.5 * run) / len(lst), k, lst[i:i + run])
             for k, lst in enumerate(lists) for i in range(0, len(lst), run)]
    return [fn for _, _, part in sorted(keyed, key=lambda e: e[:2]) for fn in part]


def _ds(start, size, align):
    return pl.ds(start if isinstance(start, int) else pl.multiple_of(start, align), size)


def _start(queue, src, dst, sem):
    pltpu.make_async_copy(src, dst, sem).start(priority=queue)


def _wait(buf, sem):
    pltpu.make_async_copy(buf, buf, sem).wait()


def _tree_sum(xs):
    while len(xs) > 1:
        xs = [xs[i] + xs[i + 1] if i + 1 < len(xs) else xs[i] for i in range(0, len(xs), 2)]
    return xs[0]


def _rows_dot(w, col):
    prod = w.astype(f32) * jnp.tile(col, (1, w.shape[1] // 128))
    return _tree_sum([prod[i:i + 8] for i in range(0, w.shape[0], 8)])


def _columns(v):
    eye = (jax.lax.broadcasted_iota(jnp.int32, (128, 128), 0)
           == jax.lax.broadcasted_iota(jnp.int32, (128, 128), 1))
    return jnp.broadcast_to(jnp.sum(jnp.where(eye, v, 0.0), axis=1, keepdims=True), (128, 128))


def _kernel(x_hbm, kT, vT, wq, wo, wr_hbm, wg, wu, wd, gw_hbm, out_ref,
            x_v, wr_v, gw_v, kv_b, wq0_b, wq_b, gu_b, out_b,
            x_c, q_c, o_c, h_c, s_s, p_s, o_s, q_s, gu_s, a_s, sems):
    def sem(i):
        return sems.at[NSEM + i]

    def kv_copies(h, piece, t):
        w, r, n, cols = piece
        if cols == list(range(cols[0], cols[0] + len(cols))):
            spans = [(r, n, cols[0] * U, len(cols) * U)]
        else:
            spans = [(g, 8, c * U, U) for g in range(r, r + n, 8) for c in cols]
        return [pltpu.make_async_copy((kT, vT)[w].at[_ds(h * DH + g, m, 8), pl.ds(BASE + c, width)],
                                      kv_b.at[h % 2, w, pl.ds(PAD + g, m), pl.ds(c, width)], sems.at[t % NSEM])
                for g, m, c, width in spans]

    def kv_start(h, piece, t):
        for copy in kv_copies(h, piece, t):
            copy.start(priority=1)

    def stream(h, pieces, requests, tasks):
        for t in range(T):
            for copy in kv_copies(h, pieces[t], t):
                copy.wait()
            for fn in requests.get(t, []):
                fn()
            nxt = t + AHEAD - T
            if nxt < 0:
                kv_start(h, pieces[t + AHEAD], t + AHEAD)
            elif pieces is FIRST or (pieces is MID and MID[nxt] == LAST[nxt]):
                kv_start(h + 1, MID[nxt], nxt)
            elif pieces is MID:
                pl.when(h < H - 2)(lambda: kv_start(h + 1, MID[nxt], nxt))
                pl.when(h == H - 2)(lambda: kv_start(H - 1, LAST[nxt], nxt))
            for fn in tasks.get(t, []):
                fn()

    def attention(h, pieces):
        def piece(w, r0, rows, cols):
            cuts = sorted({r0, r0 + rows} | {e for e in (0, DH) if r0 < e < r0 + rows})
            for r, end in zip(cuts, cuts[1:]):
                slot = (h + r // DH % 2) % 2
                blks = [(kv_b[h % 2, w, PAD + r:PAD + end, c * U:(c + 1) * U], pl.ds(c * U, U)) for c in cols]
                if w == 0:
                    q = q_c[_ds(h * DH + r, end - r, 8)]
                    for blk, c in blks:
                        s = _rows_dot(blk, q)
                        s_s[slot, :, c] = s if r % DH == 0 else s_s[slot, :, c] + s
                else:
                    prods = [blk.astype(f32) * jnp.tile(p_s[slot, :, c], ((end - r) // 8, 1)) for blk, c in blks]
                    o = _tree_sum([v[:, i:i + 128] for v in prods for i in range(0, U, 128)])
                    o_s[PAD + r:PAD + end] = o if cols == SWEEPS[1][0] else o_s[PAD + r:PAD + end] + o

        def softmax():
            s = jnp.sum(s_s[h % 2], axis=0, keepdims=True) * DH ** -0.5
            e = jnp.exp(s - jnp.max(s, axis=1, keepdims=True))
            p_s[h % 2] = jnp.broadcast_to(e * (1.0 / jnp.sum(e, axis=1, keepdims=True)), (8, W))

        def finish():
            r, end = pieces[T // 2][1], sum(pieces[-1][1:3])
            o = jnp.sum(o_s[PAD + r:PAD + end], axis=1, keepdims=True)
            o_c[_ds(h * DH + r, end - r, 8)] = jnp.broadcast_to(o, (end - r, 128))

        fns = [[lambda p=p: piece(*p)] for p in pieces]
        fns[T // 2 - 1].append(softmax)
        fns[T - 1].append(finish)
        return fns

    def first_unit(i, r):
        _start(0, wq.at[_ds(r, 8, 8), pl.ds(i * U, U)], wq0_b.at[i, _ds(r, 8, 8)], sem(i))

    first_stride = 8 * 31

    def first_units(i):
        return [lambda r=k * first_stride % D: first_unit(i, r) for k in range(D // 8)]

    def first_tasks(i):
        def part(r):
            v = _rows_dot(wq0_b[i, r:r + 32], x_c[r:r + 32])
            q_s[0, :, :U] = v if r == 0 else q_s[0, :, :U] + v

        def put(c):
            q_c[i * U + c:i * U + c + 128] = _columns(jnp.sum(q_s[0, :, c:c + 128], axis=0, keepdims=True))

        return ([lambda: _wait(wq0_b.at[i], sem(i))] + [lambda r=r: part(r) for r in range(0, D, 32)]
                + _spaced([lambda c=c: put(c) for c in range(0, U, 128)]))

    def q_units(i):
        def unit(r, c):
            _start(0, wq.at[_ds(i % 2 * QR + r, 8, 8), _ds(i // 2 * QC + c, U, U)],
                   wq_b.at[i % 2, pl.ds(r, 8), pl.ds(c, U)], sem(i % 2))
        return [lambda r=8 * 7 * k % QR, c=c: unit(r, c) for k in range(QR // 8) for c in (0, U)]

    def q_tasks(i):
        def part(r):
            v = _rows_dot(wq_b[i % 2, r:r + 16], x_c[_ds(i % 2 * QR + r, 16, 16)])
            q_s[i % 2] = v if r == 0 else q_s[i % 2] + v

        def put(c):
            @pl.when(i % 2 == 1)
            def _():
                q = jnp.sum(q_s[0, :, c:c + 128] + q_s[1, :, c:c + 128], axis=0, keepdims=True)
                q_c[_ds(i // 2 * QC + c, 128, 128)] = _columns(q)

        return ([lambda: _wait(wq_b.at[i % 2], sem(i % 2))] + [lambda r=r: part(r) for r in range(0, QR, 16)]
                + _spaced([lambda c=c: put(c) for c in range(0, QC, 128)]))

    def gu_units(i):
        def unit(m, r, c):
            _start(0, (wg, wu)[m].at[_ds((i - NQ) * GR + r, 8, 8), pl.ds(c, U)],
                   gu_b.at[i % 2, m, pl.ds(r, 8), pl.ds(c, U)], sem(i % 2))
        return _merge([[lambda m=m, r=r, c=c: unit(m, r, c) for r in range(0, GR, 8) for c in range(0, F, U)]
                       for m in range(2)])

    def gu_tasks(i):
        def part(m, r, c):
            gu_s[m, :, c:c + U] += _rows_dot(gu_b[i % 2, m, r:r + 32, c:c + U], x_c[_ds((i - NQ) * GR + r, 32, 32)])

        return [lambda: _wait(gu_b.at[i % 2], sem(i % 2))] + [
            lambda m=m, r=r, c=c: part(m, r, c) for m in range(2) for r in range(0, GR, 32) for c in range(0, F, U)]

    def swiglu(c):
        g, u = [jnp.sum(gu_s[m, :, c:c + 128], axis=0, keepdims=True) for m in range(2)]
        h_c[c:c + 128] = _columns(jax.nn.silu(g) * u)

    def out_parts(i):
        j = i - NQ - NG
        return [(wo, o_c, j * DH, DH, 0, 0), (wo, o_c, (NO + j) * DH - LAG, DH, DH, 0), (wd, h_c, j * DR, DR, 2 * DH, 1)]

    def part_units(i, part, r0, n, queue, s):
        src, _, row0, _, off, _ = part

        def unit(r, spans):
            for g, c, tiles in spans:
                cols = pl.ds(128 * c, 128 * tiles)
                _start(queue, src.at[_ds(row0 + r + 8 * g, 8, 8), cols], out_b.at[i % 2, pl.ds(off + r + 8 * g, 8), cols], s)
        return [lambda r=r, spans=spans: unit(r, spans) for r in range(r0, r0 + n, 32) for spans in SPLIT]

    def out_units(i):
        return _merge([part_units(i, p, 0, p[3], 0, sem(i % 2)) for p in out_parts(i)])

    def out_tasks(i):
        def part(p, r):
            _, col, row0, _, off, acc = p
            a_s[acc] += _rows_dot(out_b[i % 2, off + r:off + r + 32], col[_ds(row0 + r, 32, 32)])

        return [lambda: _wait(out_b.at[i % 2], sem(i % 2))] + [
            lambda p=p, r=r: part(p, r) for p in out_parts(i) for r in range(0, p[3], 32)]

    small = [pltpu.make_async_copy(x_hbm, x_v, sem(2)),
             pltpu.make_async_copy(gw_hbm, gw_v, sem(3)),
             pltpu.make_async_copy(wr_hbm, wr_v, sem(4))]
    for t in range(AHEAD):
        kv_start(0, FIRST[t], t)
        if t % 8 == 0:
            first_units(0)[t // 8]()
        if t == 4:
            for copy in small:
                copy.start()

    def warm(k, carry):
        first_unit(0, k * first_stride % D)
        return carry

    jax.lax.fori_loop(pl.cdiv(AHEAD, 8), WARM, warm, 0)

    def setup():
        for copy in small:
            copy.wait()
        a_s[...] = jnp.zeros(a_s.shape, f32)
        gu_s[...] = jnp.zeros(gu_s.shape, f32)

    def x_columns(c):
        x_c[c:c + 128] = _columns(x_v[0][:, c:c + 128].astype(f32))

    tasks = _place({}, [setup] + [lambda c=c: x_columns(c) for c in range(0, D, 128)], 2, FIRST_END)
    _place(tasks, first_tasks(0), FIRST_END + 10, FIRST_END + 20)
    third = 3 * (FIRST_END + 20)
    for t, fns in enumerate(attention(0, FIRST)):
        third = max(third + 1, 3 * t)
        tasks.setdefault(min(third // 3, T - 1), []).extend(fns)
    requests = _place(_place({}, first_units(0)[WARM:], 0, FIRST_END), first_units(1), FIRST_END, T)
    stream(0, FIRST, requests, tasks)

    def heads(lo, hi, units, consume, consume_first):
        def body(h, carry):
            tasks = dict(enumerate(attention(h, MID)))
            _place(tasks, [fn and (lambda fn=fn: pl.when(h == lo)(fn)) for fn in consume_first], LANDED, T - 2)
            _place(tasks, [fn and (lambda fn=fn: pl.when(h > lo)(fn)) for fn in consume(h)], LANDED, T - 2)
            stream(h, MID, _place({}, units(h + 1), 0, T), tasks)
            return carry
        jax.lax.fori_loop(lo, hi, body, 0)

    heads(1, NQ - 1, q_units, q_tasks, first_tasks(1))
    heads(NQ - 1, NQ + NG - 1, gu_units, gu_tasks, q_tasks(NQ - 1))
    heads(NQ + NG - 1, H - 1, out_units, out_tasks,
          gu_tasks(NQ + NG - 1) + _spaced([lambda c=c: swiglu(c) for c in range(0, F, 128)]))

    low, high, ffn = out_parts(H)
    high = high[:4] + (DH - LAG,) + high[5:]
    tail = [(0, high, LAG, 160), (1, high, 0, LAG), (1, low, 0, 64), (0, high, LAG + 160, 32),
            (1, low, 64, 32), (1, low, 96, 32)]

    def tail_units(queue):
        return [fn for k, (q, p, r, n) in enumerate(tail) if q == queue
                for fn in part_units(H, p, r, n, q, sem(6 + k))]

    requests = _place({}, part_units(H, ffn, 0, DR, 0, sem(5)) + tail_units(0), 0, LAST_END)
    _place(requests, tail_units(1), T - AHEAD, T - AHEAD + 8)
    mix = {}

    def ffn_branch():
        _wait(out_b.at[0, pl.ds(ffn[4], DR)], sem(5))
        y = a_s[1] + _rows_dot(out_b[0, ffn[4]:ffn[4] + DR], h_c[ffn[2]:ffn[2] + DR])
        y = jnp.sum(y, axis=0, keepdims=True)
        x = x_v[0].astype(f32)
        gate = jax.nn.sigmoid(jnp.sum(x * gw_v[...].astype(f32).reshape(1, D), axis=-1, keepdims=True))
        route = jax.nn.sigmoid(jnp.sum(x * wr_v[...].astype(f32).reshape(1, D), axis=-1, keepdims=True))
        mix['gate'] = gate
        mix['ffn'] = (1.0 - gate) * (x + (x * 0.0 + y * route))

    tasks = _place(dict(enumerate(attention(H - 1, LAST))), out_tasks(H - 1) + [ffn_branch], LANDED, 48)
    stream(H - 1, LAST, requests, tasks)

    row0 = jax.lax.broadcasted_iota(jnp.int32, (8, D), 0) == 0
    acc = mix['gate'] * a_s[0] + jnp.where(row0, mix['ffn'], 0.0)
    for k, (_, (_, _, first, _, off, _), r, n) in enumerate(tail):
        col = mix['gate'] * o_c[first + r:first + r + n]
        _wait(out_b.at[0, pl.ds(off + r, n)], sem(6 + k))
        acc = acc + _rows_dot(out_b[0, off + r:off + r + n], col)
    out_ref[0] = jnp.sum(acc, axis=0, keepdims=True).astype(bf16)


@jax.jit
def pallas_gated_mix__sliding_block_cached__moe_arch_mod__decode_kernel(
        A_x, A_k_cache, A_v_cache, A_wq, A_wo, B_x, B_w_r, B_w_gate, B_w_up, B_w_down, gate_w):
    del B_x
    kT = jnp.swapaxes(A_k_cache, 2, 3).reshape(H * DH, SK)
    vT = jnp.swapaxes(A_v_cache, 2, 3).reshape(H * DH, SK)
    vmem = pltpu.VMEM
    return pl.pallas_call(
        _kernel,
        out_shape=jax.ShapeDtypeStruct((1, 1, D), bf16),
        in_specs=[pl.BlockSpec(memory_space=pl.ANY)] * 10,
        out_specs=pl.BlockSpec(memory_space=pltpu.VMEM),
        scratch_shapes=[
            vmem((1, 1, D), bf16), vmem((D,), bf16), vmem((D,), bf16),
            vmem((2, 2, DH + 2 * PAD, W), bf16), vmem((2, D, U), bf16), vmem((2, QR, QC), bf16),
            vmem((2, 2, GR, F), bf16), vmem((2, 2 * DH + DR, D), bf16),
            vmem((D, 128), f32), vmem((H * DH, 128), f32), vmem((H * DH, 128), f32), vmem((F, 128), f32),
            vmem((2, 8, W), f32), vmem((2, 8, W), f32), vmem((PAD + DH, 128), f32),
            vmem((2, 8, QC), f32), vmem((2, 8, F), f32), vmem((2, 8, D), f32),
            pltpu.SemaphoreType.DMA((NSEM + 12,)),
        ],
        compiler_params=pltpu.CompilerParams(
            vmem_limit_bytes=64 * 1024 * 1024,
            disable_semaphore_checks=True,
            disable_bounds_checks=True,
        ),
        name="gated_mix_decode",
    )(A_x, kT, vT, A_wq, A_wo, B_w_r, B_w_gate, B_w_up, B_w_down, gate_w)
```

```python
import jax
import jax.numpy as jnp
import jax.experimental.pallas as pl
import jax.experimental.pallas.tpu as pltpu

H, DH, SK, D, F = 32, 192, 32768, 640, 1536
W = min(4096, max(256, SK // 4))
BASE = SK - W
U = 512

KR = 48
COL_ORDER = (0, 3, 4, 7, 6, 5, 2, 1)
SHIFT = (40, -16)
PAD = KR
AHEAD = 32
NSEM = 32
assert 0 <= SHIFT[0] < KR and -KR < SHIFT[1] <= 0


def _pieces(first=False, last=False):
    out = []
    for w in range(2):
        edges = list(range(SHIFT[w], SHIFT[w] + DH + 1, KR))
        edges[0] = 0 if first else edges[0]
        edges[-1] = DH if last else edges[-1]
        out += [(w, r0, r1, c * U) for c in COL_ORDER for r0, r1 in zip(edges, edges[1:])]
    return out


FIRST, MID, LAST = _pieces(first=True), _pieces(), _pieces(last=True)
T = len(MID)

QR, QC = D // 2, 2 * U
NQ = 2 * H * DH // QC
GR = 128
NG = D // GR
NO = H // 2
DR = F // NO
LAG = 64
LANDED = 14
FIRST_END = 22
LAST_END = 57
assert NQ + NG + NO == H + 1

SPLIT = [[(0, 0, 4)], [(0, 4, 1), (1, 0, 3)], [(1, 3, 2), (2, 0, 2)], [(2, 2, 3), (3, 0, 1)], [(3, 1, 4)]]

f32 = jnp.float32
bf16 = jnp.bfloat16


def _place(schedule, fns, t0, t1):
    for i, fn in enumerate(fns):
        if fn is not None:
            schedule.setdefault(t0 + int((i + 0.5) * (t1 - t0) / len(fns)), []).append(fn)
    return schedule


def _spaced(fns):
    return [g for fn in fns for g in [fn] + [None] * 5]


def _merge(lists, run=2):
    keyed = [((i + 0.5 * run) / len(lst), k, lst[i:i + run])
             for k, lst in enumerate(lists) for i in range(0, len(lst), run)]
    return [fn for _, _, part in sorted(keyed, key=lambda e: e[:2]) for fn in part]


def _ds(start, size, align):
    return pl.ds(start if isinstance(start, int) else pl.multiple_of(start, align), size)


def _start(queue, src, dst, sem):
    pltpu.make_async_copy(src, dst, sem).start(priority=queue)


def _wait(buf, sem):
    pltpu.make_async_copy(buf, buf, sem).wait()


def _tree_sum(xs):
    while len(xs) > 1:
        xs = [xs[i] + xs[i + 1] if i + 1 < len(xs) else xs[i] for i in range(0, len(xs), 2)]
    return xs[0]


def _rows_dot(w, col):
    prod = w.astype(f32) * jnp.tile(col, (1, w.shape[1] // 128))
    return _tree_sum([prod[i:i + 8] for i in range(0, w.shape[0], 8)])


def _columns(v):
    eye = (jax.lax.broadcasted_iota(jnp.int32, (128, 128), 0)
           == jax.lax.broadcasted_iota(jnp.int32, (128, 128), 1))
    return jnp.broadcast_to(jnp.sum(jnp.where(eye, v, 0.0), axis=1, keepdims=True), (128, 128))


def _kernel(x_hbm, kT, vT, wq, wo, wr_hbm, wg, wu, wd, gw_hbm, out_ref,
            x_v, wr_v, gw_v, kv_b, wq0_b, wq_b, gu_b, out_b,
            x_c, q_c, o_c, h_c, s_s, p_s, o_s, q_s, gu_s, a_s, sems):
    def sem(i):
        return sems.at[NSEM + i]

    def kv_copy(h, piece, t):
        w, r0, r1, c = piece
        return pltpu.make_async_copy((kT, vT)[w].at[_ds(h * DH + r0, r1 - r0, 8), _ds(BASE + c, U, U)],
                                     kv_b.at[h % 2, w, pl.ds(PAD + r0, r1 - r0), _ds(c, U, U)], sems.at[t])

    def stream(h, pieces, requests, tasks):
        for t in range(T):
            kv_copy(h, pieces[t], t % NSEM).wait()
            for fn in requests.get(t, []):
                fn()
            nxt, slot = t + AHEAD - T, (t + AHEAD) % NSEM
            if nxt < 0:
                kv_copy(h, pieces[t + AHEAD], slot).start(priority=1)
            elif pieces is FIRST or (pieces is MID and MID[nxt] == LAST[nxt]):
                kv_copy(h + 1, MID[nxt], slot).start(priority=1)
            elif pieces is MID:
                pl.when(h < H - 2)(lambda: kv_copy(h + 1, MID[nxt], slot).start(priority=1))
                pl.when(h == H - 2)(lambda: kv_copy(H - 1, LAST[nxt], slot).start(priority=1))
            for fn in tasks.get(t, []):
                fn()

    def attention(h, pieces):
        def piece(w, r0, r1, c):
            cuts = [r0] + [e for e in (0, DH) if r0 < e < r1] + [r1]
            for r, end in zip(cuts, cuts[1:]):
                slot = (h + r // DH % 2) % 2
                blk = kv_b[h % 2, w, PAD + r:PAD + end, c:c + U]
                if w == 0:
                    s = _rows_dot(blk, q_c[_ds(h * DH + r, end - r, 8)])
                    s_s[slot, :, c:c + U] = s if r % DH == 0 else s_s[slot, :, c:c + U] + s
                else:
                    prod = blk.astype(f32) * jnp.tile(p_s[slot, :, c:c + U], ((end - r) // 8, 1))
                    o = _tree_sum([prod[:, i:i + 128] for i in range(0, U, 128)])
                    o_s[PAD + r:PAD + end] = o if c == COL_ORDER[0] * U else o_s[PAD + r:PAD + end] + o

        def softmax():
            s = jnp.sum(s_s[h % 2], axis=0, keepdims=True) * DH ** -0.5
            e = jnp.exp(s - jnp.max(s, axis=1, keepdims=True))
            p_s[h % 2] = jnp.broadcast_to(e * (1.0 / jnp.sum(e, axis=1, keepdims=True)), (8, W))

        def finish():
            r, end = pieces[T // 2][1], pieces[-1][2]
            o = jnp.sum(o_s[PAD + r:PAD + end], axis=1, keepdims=True)
            o_c[_ds(h * DH + r, end - r, 8)] = jnp.broadcast_to(o, (end - r, 128))

        fns = [[lambda p=p: piece(*p)] for p in pieces]
        fns[T // 2 - 1].append(softmax)
        fns[T - 1].append(finish)
        return fns

    def first_unit(i, r):
        _start(0, wq.at[_ds(r, 8, 8), pl.ds(i * U, U)], wq0_b.at[i, _ds(r, 8, 8)], sem(i))

    first_stride = 8 * 31

    def first_units(i):
        return [lambda r=k * first_stride % D: first_unit(i, r) for k in range(D // 8)]

    def first_tasks(i):
        def part(r):
            v = _rows_dot(wq0_b[i, r:r + 32], x_c[r:r + 32])
            q_s[0, :, :U] = v if r == 0 else q_s[0, :, :U] + v

        def put(c):
            q_c[i * U + c:i * U + c + 128] = _columns(jnp.sum(q_s[0, :, c:c + 128], axis=0, keepdims=True))

        return ([lambda: _wait(wq0_b.at[i], sem(i))] + [lambda r=r: part(r) for r in range(0, D, 32)]
                + _spaced([lambda c=c: put(c) for c in range(0, U, 128)]))

    def q_units(i):
        def unit(r, c):
            _start(0, wq.at[_ds(i % 2 * QR + r, 8, 8), _ds(i // 2 * QC + c, U, U)],
                   wq_b.at[i % 2, pl.ds(r, 8), pl.ds(c, U)], sem(i % 2))
        return [lambda r=8 * 33 * k % QR, c=c: unit(r, c) for k in range(QR // 8) for c in (0, U)]

    def q_tasks(i):
        def part(r):
            v = _rows_dot(wq_b[i % 2, r:r + 16], x_c[_ds(i % 2 * QR + r, 16, 16)])
            q_s[i % 2] = v if r == 0 else q_s[i % 2] + v

        def put(c):
            @pl.when(i % 2 == 1)
            def _():
                q = jnp.sum(q_s[0, :, c:c + 128] + q_s[1, :, c:c + 128], axis=0, keepdims=True)
                q_c[_ds(i // 2 * QC + c, 128, 128)] = _columns(q)

        return ([lambda: _wait(wq_b.at[i % 2], sem(i % 2))] + [lambda r=r: part(r) for r in range(0, QR, 16)]
                + _spaced([lambda c=c: put(c) for c in range(0, QC, 128)]))

    def gu_units(i):
        def unit(m, r, c):
            _start(0, (wg, wu)[m].at[_ds((i - NQ) * GR + r, 8, 8), pl.ds(c, U)],
                   gu_b.at[i % 2, m, pl.ds(r, 8), pl.ds(c, U)], sem(i % 2))
        return _merge([[lambda m=m, r=r, c=c: unit(m, r, c) for r in range(0, GR, 8) for c in range(0, F, U)]
                       for m in range(2)])

    def gu_tasks(i):
        def part(m, r, c):
            gu_s[m, :, c:c + U] += _rows_dot(gu_b[i % 2, m, r:r + 32, c:c + U], x_c[_ds((i - NQ) * GR + r, 32, 32)])

        return [lambda: _wait(gu_b.at[i % 2], sem(i % 2))] + [
            lambda m=m, r=r, c=c: part(m, r, c) for m in range(2) for r in range(0, GR, 32) for c in range(0, F, U)]

    def swiglu(c):
        g, u = [jnp.sum(gu_s[m, :, c:c + 128], axis=0, keepdims=True) for m in range(2)]
        h_c[c:c + 128] = _columns(jax.nn.silu(g) * u)

    def out_parts(i):
        j = i - NQ - NG
        return [(wo, o_c, j * DH, DH, 0, 0), (wo, o_c, (NO + j) * DH - LAG, DH, DH, 0), (wd, h_c, j * DR, DR, 2 * DH, 1)]

    def part_units(i, part, r0, n, queue, s):
        src, _, row0, _, off, _ = part

        def unit(r, spans):
            for g, c, tiles in spans:
                cols = pl.ds(128 * c, 128 * tiles)
                _start(queue, src.at[_ds(row0 + r + 8 * g, 8, 8), cols], out_b.at[i % 2, pl.ds(off + r + 8 * g, 8), cols], s)
        return [lambda r=r, spans=spans: unit(r, spans) for r in range(r0, r0 + n, 32) for spans in SPLIT]

    def out_units(i):
        return _merge([part_units(i, p, 0, p[3], 0, sem(i % 2)) for p in out_parts(i)])

    def out_tasks(i):
        def part(p, r):
            _, col, row0, _, off, acc = p
            a_s[acc] += _rows_dot(out_b[i % 2, off + r:off + r + 32], col[_ds(row0 + r, 32, 32)])

        return [lambda: _wait(out_b.at[i % 2], sem(i % 2))] + [
            lambda p=p, r=r: part(p, r) for p in out_parts(i) for r in range(0, p[3], 32)]

    small = [pltpu.make_async_copy(x_hbm, x_v, sem(2)),
             pltpu.make_async_copy(gw_hbm, gw_v, sem(3)),
             pltpu.make_async_copy(wr_hbm, wr_v, sem(4))]
    per_col = DH // KR
    order_bits = sum(c << (3 * k) for k, c in enumerate(COL_ORDER))

    def warm(k, carry=None):
        c = ((order_bits >> (3 * k)) & 7) * U
        for e in range(per_col):
            kv_copy(0, FIRST[e][:3] + (c,), per_col * k + e).start(priority=1)
            if e % 2 == 0:
                first_unit(0, (per_col // 2 * k + e // 2) * first_stride % D)

    warm(0)
    for copy in small:
        copy.start()
    jax.lax.fori_loop(1, AHEAD // per_col, warm, None)

    def setup():
        for copy in small:
            copy.wait()
        a_s[...] = jnp.zeros(a_s.shape, f32)
        gu_s[...] = jnp.zeros(gu_s.shape, f32)

    def x_columns(c):
        x_c[c:c + 128] = _columns(x_v[0][:, c:c + 128].astype(f32))

    tasks = _place({}, [setup] + [lambda c=c: x_columns(c) for c in range(0, D, 128)], 2, FIRST_END)
    _place(tasks, first_tasks(0), FIRST_END + 10, FIRST_END + 20)
    third = 3 * (FIRST_END + 20)
    for t, fns in enumerate(attention(0, FIRST)):
        third = max(third + 1, 3 * t)
        tasks.setdefault(min(third // 3, T - 1), []).extend(fns)
    requests = _place(_place({}, first_units(0)[AHEAD // 2:], 0, FIRST_END), first_units(1), FIRST_END, T)
    stream(0, FIRST, requests, tasks)

    def passes(lo, hi, units, consume, consume_first):
        def body(h, carry):
            tasks = dict(enumerate(attention(h, MID)))
            _place(tasks, [fn and (lambda fn=fn: pl.when(h == lo)(fn)) for fn in consume_first], LANDED, T - 2)
            _place(tasks, [fn and (lambda fn=fn: pl.when(h > lo)(fn)) for fn in consume(h)], LANDED, T - 2)
            stream(h, MID, _place({}, units(h + 1), 0, T), tasks)
            return carry
        jax.lax.fori_loop(lo, hi, body, 0)

    passes(1, NQ - 1, q_units, q_tasks, first_tasks(1))
    passes(NQ - 1, NQ + NG - 1, gu_units, gu_tasks, q_tasks(NQ - 1))
    passes(NQ + NG - 1, H - 1, out_units, out_tasks,
           gu_tasks(NQ + NG - 1) + _spaced([lambda c=c: swiglu(c) for c in range(0, F, 128)]))

    low, high, ffn = out_parts(H)
    high = high[:4] + (DH - LAG,) + high[5:]
    tail = [(0, high, LAG, 160), (1, high, 0, LAG), (1, low, 0, 64), (0, high, LAG + 160, 32),
            (1, low, 64, 32), (1, low, 96, 32)]

    def tail_units(queue):
        return [fn for k, (q, p, r, n) in enumerate(tail) if q == queue
                for fn in part_units(H, p, r, n, q, sem(6 + k))]

    requests = _place({}, part_units(H, ffn, 0, DR, 0, sem(5)) + tail_units(0), 0, LAST_END)
    _place(requests, tail_units(1), T - AHEAD, T - AHEAD + 8)
    mix = {}

    def ffn_branch():
        _wait(out_b.at[0, pl.ds(ffn[4], DR)], sem(5))
        y = a_s[1] + _rows_dot(out_b[0, ffn[4]:ffn[4] + DR], h_c[ffn[2]:ffn[2] + DR])
        y = jnp.sum(y, axis=0, keepdims=True)
        x = x_v[0].astype(f32)
        gate = jax.nn.sigmoid(jnp.sum(x * gw_v[...].astype(f32).reshape(1, D), axis=-1, keepdims=True))
        route = jax.nn.sigmoid(jnp.sum(x * wr_v[...].astype(f32).reshape(1, D), axis=-1, keepdims=True))
        mix['gate'] = gate
        mix['ffn'] = (1.0 - gate) * (x + (x * 0.0 + y * route))

    tasks = _place(dict(enumerate(attention(H - 1, LAST))), out_tasks(H - 1) + [ffn_branch], LANDED, 48)
    stream(H - 1, LAST, requests, tasks)

    row0 = jax.lax.broadcasted_iota(jnp.int32, (8, D), 0) == 0
    acc = mix['gate'] * a_s[0] + jnp.where(row0, mix['ffn'], 0.0)
    for k, (_, (_, _, first, _, off, _), r, n) in enumerate(tail):
        col = mix['gate'] * o_c[first + r:first + r + n]
        _wait(out_b.at[0, pl.ds(off + r, n)], sem(6 + k))
        acc = acc + _rows_dot(out_b[0, off + r:off + r + n], col)
    out_ref[0] = jnp.sum(acc, axis=0, keepdims=True).astype(bf16)


@jax.jit
def pallas_gated_mix__sliding_block_cached__moe_arch_mod__decode_kernel(
        A_x, A_k_cache, A_v_cache, A_wq, A_wo, B_x, B_w_r, B_w_gate, B_w_up, B_w_down, gate_w):
    del B_x
    kT = jnp.swapaxes(A_k_cache, 2, 3).reshape(H * DH, SK)
    vT = jnp.swapaxes(A_v_cache, 2, 3).reshape(H * DH, SK)
    vmem = pltpu.VMEM
    return pl.pallas_call(
        _kernel,
        out_shape=jax.ShapeDtypeStruct((1, 1, D), bf16),
        in_specs=[pl.BlockSpec(memory_space=pl.ANY)] * 10,
        out_specs=pl.BlockSpec(memory_space=pltpu.VMEM),
        scratch_shapes=[
            vmem((1, 1, D), bf16), vmem((D,), bf16), vmem((D,), bf16),
            vmem((2, 2, DH + 2 * PAD, W), bf16), vmem((2, D, U), bf16), vmem((2, QR, QC), bf16),
            vmem((2, 2, GR, F), bf16), vmem((2, 2 * DH + DR, D), bf16),
            vmem((D, 128), f32), vmem((H * DH, 128), f32), vmem((H * DH, 128), f32), vmem((F, 128), f32),
            vmem((2, 8, W), f32), vmem((2, 8, W), f32), vmem((PAD + DH, 128), f32),
            vmem((2, 8, QC), f32), vmem((2, 8, F), f32), vmem((2, 8, D), f32),
            pltpu.SemaphoreType.DMA((NSEM + 12,)),
        ],
        compiler_params=pltpu.CompilerParams(
            vmem_limit_bytes=64 * 1024 * 1024,
            disable_semaphore_checks=True,
            disable_bounds_checks=True,
        ),
        name="gated_mix_decode",
    )(A_x, kT, vT, A_wq, A_wo, B_w_r, B_w_gate, B_w_up, B_w_down, gate_w)
```

```python
import jax
import jax.numpy as jnp
import jax.experimental.pallas as pl
import jax.experimental.pallas.tpu as pltpu

H, DH, SK, D, F = 32, 192, 32768, 640, 1536
W = min(4096, max(256, SK // 4))
BASE = SK - W
U = 512

KR = 64
COL_PAIRS = (((0, 3), (4, 7), (6, 5), (2, 1)), ((0, 3), (4, 5), (2, 1), (6, 7)))
SHIFT = (40, -16)
PAD = KR
AHEAD = 24
NSEM = 24
assert 0 <= SHIFT[0] < KR and -KR < SHIFT[1] <= 0


def _pieces(first=False, last=False):
    out = []
    for w in range(2):
        edges = list(range(SHIFT[w], SHIFT[w] + DH + 1, KR))
        edges[0] = 0 if first else edges[0]
        edges[-1] = DH if last else edges[-1]
        out += [(w, r0, r1, c * U) for pair in COL_PAIRS[w] for r0, r1 in zip(edges, edges[1:]) for c in pair]
    return out


FIRST, MID, LAST = _pieces(first=True), _pieces(), _pieces(last=True)
T = len(MID)

QR, QC = D // 2, 2 * U
NQ = 2 * H * DH // QC
GR = 128
NG = D // GR
NO = H // 2
DR = F // NO
LAG = 64
LANDED = 10
FIRST_END = 16
LAST_END = 43
assert NQ + NG + NO == H + 1

SPLIT = [[(0, 0, 4)], [(0, 4, 1), (1, 0, 3)], [(1, 3, 2), (2, 0, 2)], [(2, 2, 3), (3, 0, 1)], [(3, 1, 4)]]

f32 = jnp.float32
bf16 = jnp.bfloat16


def _place(schedule, fns, t0, t1):
    for i, fn in enumerate(fns):
        if fn is not None:
            schedule.setdefault(t0 + int((i + 0.5) * (t1 - t0) / len(fns)), []).append(fn)
    return schedule


def _spaced(fns):
    return [g for fn in fns for g in [fn] + [None] * 5]


def _merge(lists, run=2):
    keyed = [((i + 0.5 * run) / len(lst), k, lst[i:i + run])
             for k, lst in enumerate(lists) for i in range(0, len(lst), run)]
    return [fn for _, _, part in sorted(keyed, key=lambda e: e[:2]) for fn in part]


def _ds(start, size, align):
    return pl.ds(start if isinstance(start, int) else pl.multiple_of(start, align), size)


def _start(queue, src, dst, sem):
    pltpu.make_async_copy(src, dst, sem).start(priority=queue)


def _wait(buf, sem):
    pltpu.make_async_copy(buf, buf, sem).wait()


def _tree_sum(xs):
    while len(xs) > 1:
        xs = [xs[i] + xs[i + 1] if i + 1 < len(xs) else xs[i] for i in range(0, len(xs), 2)]
    return xs[0]


def _rows_dot(w, col):
    prod = w.astype(f32) * jnp.tile(col, (1, w.shape[1] // 128))
    return _tree_sum([prod[i:i + 8] for i in range(0, w.shape[0], 8)])


def _columns(v):
    eye = (jax.lax.broadcasted_iota(jnp.int32, (128, 128), 0)
           == jax.lax.broadcasted_iota(jnp.int32, (128, 128), 1))
    return jnp.broadcast_to(jnp.sum(jnp.where(eye, v, 0.0), axis=1, keepdims=True), (128, 128))


def _kernel(x_hbm, kT, vT, wq, wo, wr_hbm, wg, wu, wd, gw_hbm, out_ref,
            x_v, wr_v, gw_v, kv_b, wq0_b, wq_b, gu_b, out_b,
            x_c, q_c, o_c, h_c, s_s, p_s, o_s, q_s, gu_s, a_s, sems):
    def sem(i):
        return sems.at[NSEM + i]

    def kv_copy(h, piece, t):
        w, r0, r1, c = piece
        return pltpu.make_async_copy((kT, vT)[w].at[_ds(h * DH + r0, r1 - r0, 8), _ds(BASE + c, U, U)],
                                     kv_b.at[h % 2, w, pl.ds(PAD + r0, r1 - r0), _ds(c, U, U)], sems.at[t])

    def stream(h, pieces, requests, tasks):
        for t in range(T):
            kv_copy(h, pieces[t], t % NSEM).wait()
            for fn in requests.get(t, []):
                fn()
            nxt, slot = t + AHEAD - T, (t + AHEAD) % NSEM
            if nxt < 0:
                kv_copy(h, pieces[t + AHEAD], slot).start(priority=1)
            elif pieces is FIRST or (pieces is MID and MID[nxt] == LAST[nxt]):
                kv_copy(h + 1, MID[nxt], slot).start(priority=1)
            elif pieces is MID:
                pl.when(h < H - 2)(lambda: kv_copy(h + 1, MID[nxt], slot).start(priority=1))
                pl.when(h == H - 2)(lambda: kv_copy(H - 1, LAST[nxt], slot).start(priority=1))
            for fn in tasks.get(t, []):
                fn()

    def attention(h, pieces):
        def piece(w, r0, r1, c):
            cuts = [r0] + [e for e in (0, DH) if r0 < e < r1] + [r1]
            for r, end in zip(cuts, cuts[1:]):
                slot = (h + r // DH % 2) % 2
                blk = kv_b[h % 2, w, PAD + r:PAD + end, c:c + U]
                if w == 0:
                    s = _rows_dot(blk, q_c[_ds(h * DH + r, end - r, 8)])
                    s_s[slot, :, c:c + U] = s if r % DH == 0 else s_s[slot, :, c:c + U] + s
                else:
                    prod = blk.astype(f32) * jnp.tile(p_s[slot, :, c:c + U], ((end - r) // 8, 1))
                    o = _tree_sum([prod[:, i:i + 128] for i in range(0, U, 128)])
                    o_s[PAD + r:PAD + end] = o if c == COL_PAIRS[1][0][0] * U else o_s[PAD + r:PAD + end] + o

        def softmax():
            s = jnp.sum(s_s[h % 2], axis=0, keepdims=True) * DH ** -0.5
            e = jnp.exp(s - jnp.max(s, axis=1, keepdims=True))
            p_s[h % 2] = jnp.broadcast_to(e * (1.0 / jnp.sum(e, axis=1, keepdims=True)), (8, W))

        def finish():
            r, end = pieces[T // 2][1], pieces[-1][2]
            o = jnp.sum(o_s[PAD + r:PAD + end], axis=1, keepdims=True)
            o_c[_ds(h * DH + r, end - r, 8)] = jnp.broadcast_to(o, (end - r, 128))

        fns = [[lambda p=p: piece(*p)] for p in pieces]
        fns[T // 2 - 1].append(softmax)
        fns[T - 1].append(finish)
        return fns

    def first_unit(i, r):
        _start(0, wq.at[_ds(r, 8, 8), pl.ds(i * U, U)], wq0_b.at[i, _ds(r, 8, 8)], sem(i))

    first_stride = 8 * 31

    def first_units(i):
        return [lambda r=k * first_stride % D: first_unit(i, r) for k in range(D // 8)]

    def first_tasks(i):
        def part(r):
            v = _rows_dot(wq0_b[i, r:r + 32], x_c[r:r + 32])
            q_s[0, :, :U] = v if r == 0 else q_s[0, :, :U] + v

        def put(c):
            q_c[i * U + c:i * U + c + 128] = _columns(jnp.sum(q_s[0, :, c:c + 128], axis=0, keepdims=True))

        return ([lambda: _wait(wq0_b.at[i], sem(i))] + [lambda r=r: part(r) for r in range(0, D, 32)]
                + _spaced([lambda c=c: put(c) for c in range(0, U, 128)]))

    def q_units(i):
        def unit(r, c):
            _start(0, wq.at[_ds(i % 2 * QR + r, 8, 8), _ds(i // 2 * QC + c, U, U)],
                   wq_b.at[i % 2, pl.ds(r, 8), pl.ds(c, U)], sem(i % 2))
        return [lambda r=8 * 33 * k % QR, c=c: unit(r, c) for k in range(QR // 8) for c in (0, U)]

    def q_tasks(i):
        def part(r):
            v = _rows_dot(wq_b[i % 2, r:r + 16], x_c[_ds(i % 2 * QR + r, 16, 16)])
            q_s[i % 2] = v if r == 0 else q_s[i % 2] + v

        def put(c):
            @pl.when(i % 2 == 1)
            def _():
                q = jnp.sum(q_s[0, :, c:c + 128] + q_s[1, :, c:c + 128], axis=0, keepdims=True)
                q_c[_ds(i // 2 * QC + c, 128, 128)] = _columns(q)

        return ([lambda: _wait(wq_b.at[i % 2], sem(i % 2))] + [lambda r=r: part(r) for r in range(0, QR, 16)]
                + _spaced([lambda c=c: put(c) for c in range(0, QC, 128)]))

    def gu_units(i):
        def unit(m, r, c):
            _start(0, (wg, wu)[m].at[_ds((i - NQ) * GR + r, 8, 8), pl.ds(c, U)],
                   gu_b.at[i % 2, m, pl.ds(r, 8), pl.ds(c, U)], sem(i % 2))
        return _merge([[lambda m=m, r=r, c=c: unit(m, r, c) for r in range(0, GR, 8) for c in range(0, F, U)]
                       for m in range(2)])

    def gu_tasks(i):
        def part(m, r, c):
            gu_s[m, :, c:c + U] += _rows_dot(gu_b[i % 2, m, r:r + 32, c:c + U], x_c[_ds((i - NQ) * GR + r, 32, 32)])

        return [lambda: _wait(gu_b.at[i % 2], sem(i % 2))] + [
            lambda m=m, r=r, c=c: part(m, r, c) for m in range(2) for r in range(0, GR, 32) for c in range(0, F, U)]

    def swiglu(c):
        g, u = [jnp.sum(gu_s[m, :, c:c + 128], axis=0, keepdims=True) for m in range(2)]
        h_c[c:c + 128] = _columns(jax.nn.silu(g) * u)

    def out_parts(i):
        j = i - NQ - NG
        return [(wo, o_c, j * DH, DH, 0, 0), (wo, o_c, (NO + j) * DH - LAG, DH, DH, 0), (wd, h_c, j * DR, DR, 2 * DH, 1)]

    def part_units(i, part, r0, n, queue, s):
        src, _, row0, _, off, _ = part

        def unit(r, spans):
            for g, c, tiles in spans:
                cols = pl.ds(128 * c, 128 * tiles)
                _start(queue, src.at[_ds(row0 + r + 8 * g, 8, 8), cols], out_b.at[i % 2, pl.ds(off + r + 8 * g, 8), cols], s)
        return [lambda r=r, spans=spans: unit(r, spans) for r in range(r0, r0 + n, 32) for spans in SPLIT]

    def out_units(i):
        return _merge([part_units(i, p, 0, p[3], 0, sem(i % 2)) for p in out_parts(i)])

    def out_tasks(i):
        def part(p, r):
            _, col, row0, _, off, acc = p
            a_s[acc] += _rows_dot(out_b[i % 2, off + r:off + r + 32], col[_ds(row0 + r, 32, 32)])

        return [lambda: _wait(out_b.at[i % 2], sem(i % 2))] + [
            lambda p=p, r=r: part(p, r) for p in out_parts(i) for r in range(0, p[3], 32)]

    small = [pltpu.make_async_copy(x_hbm, x_v, sem(2)),
             pltpu.make_async_copy(gw_hbm, gw_v, sem(3)),
             pltpu.make_async_copy(wr_hbm, wr_v, sem(4))]
    order_bits = sum(c // U << (6 * (t // 6) + 3 * (t % 2)) for t, (_, _, _, c) in enumerate(FIRST[:AHEAD]) if t % 6 < 2)

    def warm(k, carry=None):
        for e in range(6):
            c = ((order_bits >> (6 * k + 3 * (e % 2))) & 7) * U
            kv_copy(0, FIRST[e][:3] + (c,), 6 * k + e).start(priority=1)
            if e % 3 < 2:
                first_unit(0, (4 * k + e - e // 3) * first_stride % D)

    warm(0)
    for copy in small:
        copy.start()
    jax.lax.fori_loop(1, AHEAD // 6, warm, None)

    def setup():
        for copy in small:
            copy.wait()
        a_s[...] = jnp.zeros(a_s.shape, f32)
        gu_s[...] = jnp.zeros(gu_s.shape, f32)

    def x_columns(c):
        x_c[c:c + 128] = _columns(x_v[0][:, c:c + 128].astype(f32))

    tasks = _place({}, [setup] + [lambda c=c: x_columns(c) for c in range(0, D, 128)], 2, FIRST_END)
    _place(tasks, first_tasks(0), FIRST_END + 8, FIRST_END + 15)
    third = 3 * (FIRST_END + 15)
    for t, fns in enumerate(attention(0, FIRST)):
        third = max(third + 1, 3 * t)
        tasks.setdefault(min(third // 3, T - 1), []).extend(fns)
    requests = _place(_place({}, first_units(0)[AHEAD // 6 * 4:], 0, FIRST_END), first_units(1), FIRST_END, T)
    stream(0, FIRST, requests, tasks)

    def passes(lo, hi, units, consume, consume_first):
        def body(h, carry):
            tasks = dict(enumerate(attention(h, MID)))
            _place(tasks, [fn and (lambda fn=fn: pl.when(h == lo)(fn)) for fn in consume_first], LANDED, T - 2)
            _place(tasks, [fn and (lambda fn=fn: pl.when(h > lo)(fn)) for fn in consume(h)], LANDED, T - 2)
            stream(h, MID, _place({}, units(h + 1), 0, T), tasks)
            return carry
        jax.lax.fori_loop(lo, hi, body, 0)

    passes(1, NQ - 1, q_units, q_tasks, first_tasks(1))
    passes(NQ - 1, NQ + NG - 1, gu_units, gu_tasks, q_tasks(NQ - 1))
    passes(NQ + NG - 1, H - 1, out_units, out_tasks,
           gu_tasks(NQ + NG - 1) + _spaced([lambda c=c: swiglu(c) for c in range(0, F, 128)]))

    low, high, ffn = out_parts(H)
    high = high[:4] + (DH - LAG,) + high[5:]
    tail = [(0, high, LAG, 160), (1, high, 0, LAG), (1, low, 0, 64), (0, high, LAG + 160, 32),
            (1, low, 64, 32), (1, low, 96, 32)]

    def tail_units(queue):
        return [fn for k, (q, p, r, n) in enumerate(tail) if q == queue
                for fn in part_units(H, p, r, n, q, sem(6 + k))]

    requests = _place({}, part_units(H, ffn, 0, DR, 0, sem(5)) + tail_units(0), 0, LAST_END)
    _place(requests, tail_units(1), T - AHEAD, T - AHEAD + 6)
    mix = {}

    def ffn_branch():
        _wait(out_b.at[0, pl.ds(ffn[4], DR)], sem(5))
        y = a_s[1] + _rows_dot(out_b[0, ffn[4]:ffn[4] + DR], h_c[ffn[2]:ffn[2] + DR])
        y = jnp.sum(y, axis=0, keepdims=True)
        x = x_v[0].astype(f32)
        gate = jax.nn.sigmoid(jnp.sum(x * gw_v[...].astype(f32).reshape(1, D), axis=-1, keepdims=True))
        route = jax.nn.sigmoid(jnp.sum(x * wr_v[...].astype(f32).reshape(1, D), axis=-1, keepdims=True))
        mix['gate'] = gate
        mix['ffn'] = (1.0 - gate) * (x + (x * 0.0 + y * route))

    tasks = _place(dict(enumerate(attention(H - 1, LAST))), out_tasks(H - 1) + [ffn_branch], LANDED, 36)
    stream(H - 1, LAST, requests, tasks)

    row0 = jax.lax.broadcasted_iota(jnp.int32, (8, D), 0) == 0
    acc = mix['gate'] * a_s[0] + jnp.where(row0, mix['ffn'], 0.0)
    for k, (_, (_, _, first, _, off, _), r, n) in enumerate(tail):
        col = mix['gate'] * o_c[first + r:first + r + n]
        _wait(out_b.at[0, pl.ds(off + r, n)], sem(6 + k))
        acc = acc + _rows_dot(out_b[0, off + r:off + r + n], col)
    out_ref[0] = jnp.sum(acc, axis=0, keepdims=True).astype(bf16)


@jax.jit
def pallas_gated_mix__sliding_block_cached__moe_arch_mod__decode_kernel(
        A_x, A_k_cache, A_v_cache, A_wq, A_wo, B_x, B_w_r, B_w_gate, B_w_up, B_w_down, gate_w):
    del B_x
    kT = jnp.swapaxes(A_k_cache, 2, 3).reshape(H * DH, SK)
    vT = jnp.swapaxes(A_v_cache, 2, 3).reshape(H * DH, SK)
    vmem = pltpu.VMEM
    return pl.pallas_call(
        _kernel,
        out_shape=jax.ShapeDtypeStruct((1, 1, D), bf16),
        in_specs=[pl.BlockSpec(memory_space=pl.ANY)] * 10,
        out_specs=pl.BlockSpec(memory_space=pltpu.VMEM),
        scratch_shapes=[
            vmem((1, 1, D), bf16), vmem((D,), bf16), vmem((D,), bf16),
            vmem((2, 2, DH + 2 * PAD, W), bf16), vmem((2, D, U), bf16), vmem((2, QR, QC), bf16),
            vmem((2, 2, GR, F), bf16), vmem((2, 2 * DH + DR, D), bf16),
            vmem((D, 128), f32), vmem((H * DH, 128), f32), vmem((H * DH, 128), f32), vmem((F, 128), f32),
            vmem((2, 8, W), f32), vmem((2, 8, W), f32), vmem((PAD + DH, 128), f32),
            vmem((2, 8, QC), f32), vmem((2, 8, F), f32), vmem((2, 8, D), f32),
            pltpu.SemaphoreType.DMA((NSEM + 12,)),
        ],
        compiler_params=pltpu.CompilerParams(
            vmem_limit_bytes=64 * 1024 * 1024,
            disable_semaphore_checks=True,
            disable_bounds_checks=True,
        ),
        name="gated_mix_decode",
    )(A_x, kT, vT, A_wq, A_wo, B_w_r, B_w_gate, B_w_up, B_w_down, gate_w)
```

```python
import jax
import jax.numpy as jnp
import jax.experimental.pallas as pl
import jax.experimental.pallas.tpu as pltpu

H, DH, SK, D, F = 32, 192, 32768, 640, 1536
W = min(4096, max(256, SK // 4))
BASE = SK - W
U = 512

KR = 64
COL_PAIRS = (((0, 3), (4, 7), (6, 5), (2, 1)), ((0, 3), (4, 5), (2, 1), (6, 7)))
SHIFT = (40, -16)
PAD = tuple(-s % KR for s in SHIFT)
AHEAD = 24
NSEM = 24
assert 0 <= SHIFT[0] < KR and -KR < SHIFT[1] <= 0


def _pieces(first=False, last=False):
    out = []
    for w in range(2):
        edges = list(range(SHIFT[w], SHIFT[w] + DH + 1, KR))
        edges[0] = 0 if first else edges[0]
        edges[-1] = DH if last else edges[-1]
        out += [(w, r0, r1, c * U) for pair in COL_PAIRS[w] for r0, r1 in zip(edges, edges[1:]) for c in pair]
    return out


FIRST, MID, LAST = _pieces(first=True), _pieces(), _pieces(last=True)
T = len(MID)

QR, QC = D // 2, 2 * U
NQ = 2 * H * DH // QC
GR = 128
NG = D // GR
NO = H // 2
DR = F // NO
LAG = 64
LANDED = 10
FIRST_END = 16
LAST_END = 43
assert NQ + NG + NO == H + 1

SPLIT = [[(0, 0, 4)], [(0, 4, 1), (1, 0, 3)], [(1, 3, 2), (2, 0, 2)], [(2, 2, 3), (3, 0, 1)], [(3, 1, 4)]]

f32 = jnp.float32
bf16 = jnp.bfloat16


def _place(schedule, fns, t0, t1):
    for i, fn in enumerate(fns):
        if fn is not None:
            schedule.setdefault(t0 + int((i + 0.5) * (t1 - t0) / len(fns)), []).append(fn)
    return schedule


def _spaced(fns):
    return [g for fn in fns for g in [fn] + [None] * 5]


def _merge(lists, run=2):
    keyed = [((i + 0.5 * run) / len(lst), k, lst[i:i + run])
             for k, lst in enumerate(lists) for i in range(0, len(lst), run)]
    return [fn for _, _, part in sorted(keyed, key=lambda e: e[:2]) for fn in part]


def _ds(start, size, align):
    return pl.ds(start if isinstance(start, int) else pl.multiple_of(start, align), size)


def _start(queue, src, dst, sem):
    pltpu.make_async_copy(src, dst, sem).start(priority=queue)


def _wait(buf, sem):
    pltpu.make_async_copy(buf, buf, sem).wait()


def _tree_sum(xs):
    while len(xs) > 1:
        xs = [xs[i] + xs[i + 1] if i + 1 < len(xs) else xs[i] for i in range(0, len(xs), 2)]
    return xs[0]


def _rows_dot(w, col):
    prod = w.astype(f32) * jnp.tile(col, (1, w.shape[1] // 128))
    return _tree_sum([prod[i:i + 8] for i in range(0, w.shape[0], 8)])


def _columns(v):
    eye = (jax.lax.broadcasted_iota(jnp.int32, (128, 128), 0)
           == jax.lax.broadcasted_iota(jnp.int32, (128, 128), 1))
    return jnp.broadcast_to(jnp.sum(jnp.where(eye, v, 0.0), axis=1, keepdims=True), (128, 128))


def _kernel(x_hbm, kT, vT, wq, wo, wr_hbm, wg, wu, wd, gw_hbm, out_ref,
            x_v, wr_v, gw_v, kv_b, wq0_b, wq_b, gu_b, out_b,
            x_c, q_c, o_c, h_c, s_s, p_s, o_s, q_s, gu_s, a_s, sems):
    def sem(i):
        return sems.at[NSEM + i]

    def kv_copy(h, piece, t):
        w, r0, r1, c = piece
        return pltpu.make_async_copy((kT, vT)[w].at[_ds(h * DH + r0, r1 - r0, 8), _ds(BASE + c, U, U)],
                                     kv_b.at[h % 2, w, pl.ds(PAD[w] + r0, r1 - r0), _ds(c, U, U)], sems.at[t])

    def stream(h, pieces, requests, tasks):
        for t in range(T):
            kv_copy(h, pieces[t], t % NSEM).wait()
            for fn in requests.get(t, []):
                fn()
            nxt, slot = t + AHEAD - T, (t + AHEAD) % NSEM
            if nxt < 0:
                kv_copy(h, pieces[t + AHEAD], slot).start(priority=1)
            elif pieces is FIRST or (pieces is MID and MID[nxt] == LAST[nxt]):
                kv_copy(h + 1, MID[nxt], slot).start(priority=1)
            elif pieces is MID:
                pl.when(h < H - 2)(lambda: kv_copy(h + 1, MID[nxt], slot).start(priority=1))
                pl.when(h == H - 2)(lambda: kv_copy(H - 1, LAST[nxt], slot).start(priority=1))
            for fn in tasks.get(t, []):
                fn()

    def attention(h, pieces):
        def piece(w, r0, r1, c):
            cuts = [r0] + [e for e in (0, DH) if r0 < e < r1] + [r1]
            for r, end in zip(cuts, cuts[1:]):
                slot = (h + r // DH % 2) % 2
                rows = slice(PAD[w] + r, PAD[w] + end)
                blk = kv_b[h % 2, w, rows, c:c + U]
                if w == 0:
                    s = _rows_dot(blk, q_c[_ds(h * DH + r, end - r, 8)])
                    s_s[slot, :, c:c + U] = s if r % DH == 0 else s_s[slot, :, c:c + U] + s
                else:
                    prod = blk.astype(f32) * jnp.tile(p_s[slot, :, c:c + U], ((end - r) // 8, 1))
                    o = _tree_sum([prod[:, i:i + 128] for i in range(0, U, 128)])
                    o_s[rows] = o if c == COL_PAIRS[1][0][0] * U else o_s[rows] + o

        def softmax():
            s = jnp.sum(s_s[h % 2], axis=0, keepdims=True) * DH ** -0.5
            e = jnp.exp(s - jnp.max(s, axis=1, keepdims=True))
            p_s[h % 2] = jnp.broadcast_to(e * (1.0 / jnp.sum(e, axis=1, keepdims=True)), (8, W))

        def finish():
            r, end = pieces[T // 2][1], pieces[-1][2]
            o = jnp.sum(o_s[PAD[1] + r:PAD[1] + end], axis=1, keepdims=True)
            o_c[_ds(h * DH + r, end - r, 8)] = jnp.broadcast_to(o, (end - r, 128))

        fns = [[lambda p=p: piece(*p)] for p in pieces]
        fns[T // 2 - 1].append(softmax)
        fns[T - 1].append(finish)
        return fns

    def first_unit(i, r):
        _start(0, wq.at[_ds(r, 8, 8), pl.ds(i * U, U)], wq0_b.at[i, _ds(r, 8, 8)], sem(i))

    first_stride = 8 * 31

    def first_units(i):
        return [lambda r=k * first_stride % D: first_unit(i, r) for k in range(D // 8)]

    def first_tasks(i):
        def part(r):
            v = _rows_dot(wq0_b[i, r:r + 32], x_c[r:r + 32])
            q_s[0, :, :U] = v if r == 0 else q_s[0, :, :U] + v

        def put(c):
            q_c[i * U + c:i * U + c + 128] = _columns(jnp.sum(q_s[0, :, c:c + 128], axis=0, keepdims=True))

        return ([lambda: _wait(wq0_b.at[i], sem(i))] + [lambda r=r: part(r) for r in range(0, D, 32)]
                + _spaced([lambda c=c: put(c) for c in range(0, U, 128)]))

    def q_units(i):
        def unit(r, c):
            _start(0, wq.at[_ds(i % 2 * QR + r, 8, 8), _ds(i // 2 * QC + c, U, U)],
                   wq_b.at[i % 2, pl.ds(r, 8), pl.ds(c, U)], sem(i % 2))
        return [lambda r=8 * 33 * k % QR, c=c: unit(r, c) for k in range(QR // 8) for c in (0, U)]

    def q_tasks(i):
        def part(r):
            v = _rows_dot(wq_b[i % 2, r:r + 16], x_c[_ds(i % 2 * QR + r, 16, 16)])
            q_s[i % 2] = v if r == 0 else q_s[i % 2] + v

        def put(c):
            @pl.when(i % 2 == 1)
            def _():
                q = jnp.sum(q_s[0, :, c:c + 128] + q_s[1, :, c:c + 128], axis=0, keepdims=True)
                q_c[_ds(i // 2 * QC + c, 128, 128)] = _columns(q)

        return ([lambda: _wait(wq_b.at[i % 2], sem(i % 2))] + [lambda r=r: part(r) for r in range(0, QR, 16)]
                + _spaced([lambda c=c: put(c) for c in range(0, QC, 128)]))

    def gu_units(i):
        def unit(m, r, c):
            _start(0, (wg, wu)[m].at[_ds((i - NQ) * GR + r, 8, 8), pl.ds(c, U)],
                   gu_b.at[i % 2, m, pl.ds(r, 8), pl.ds(c, U)], sem(i % 2))
        return _merge([[lambda m=m, r=r, c=c: unit(m, r, c) for r in range(0, GR, 8) for c in range(0, F, U)]
                       for m in range(2)])

    def gu_tasks(i):
        def part(m, r, c):
            gu_s[m, :, c:c + U] += _rows_dot(gu_b[i % 2, m, r:r + 32, c:c + U], x_c[_ds((i - NQ) * GR + r, 32, 32)])

        return [lambda: _wait(gu_b.at[i % 2], sem(i % 2))] + [
            lambda m=m, r=r, c=c: part(m, r, c) for m in range(2) for r in range(0, GR, 32) for c in range(0, F, U)]

    def swiglu(c):
        g, u = [jnp.sum(gu_s[m, :, c:c + 128], axis=0, keepdims=True) for m in range(2)]
        h_c[c:c + 128] = _columns(jax.nn.silu(g) * u)

    def out_parts(i):
        j = i - NQ - NG
        return [(wo, o_c, j * DH, DH, 0, 0), (wo, o_c, (NO + j) * DH - LAG, DH, DH, 0), (wd, h_c, j * DR, DR, 2 * DH, 1)]

    def part_units(i, part, r0, n, queue, s):
        src, _, row0, _, off, _ = part

        def unit(r, spans):
            for g, c, tiles in spans:
                cols = pl.ds(128 * c, 128 * tiles)
                _start(queue, src.at[_ds(row0 + r + 8 * g, 8, 8), cols], out_b.at[i % 2, pl.ds(off + r + 8 * g, 8), cols], s)
        return [lambda r=r, spans=spans: unit(r, spans) for r in range(r0, r0 + n, 32) for spans in SPLIT]

    def out_units(i):
        return _merge([part_units(i, p, 0, p[3], 0, sem(i % 2)) for p in out_parts(i)])

    def out_tasks(i):
        def part(p, r):
            _, col, row0, _, off, acc = p
            a_s[acc] += _rows_dot(out_b[i % 2, off + r:off + r + 32], col[_ds(row0 + r, 32, 32)])

        return [lambda: _wait(out_b.at[i % 2], sem(i % 2))] + [
            lambda p=p, r=r: part(p, r) for p in out_parts(i) for r in range(0, p[3], 32)]

    small = [pltpu.make_async_copy(x_hbm, x_v, sem(2)),
             pltpu.make_async_copy(gw_hbm, gw_v, sem(3)),
             pltpu.make_async_copy(wr_hbm, wr_v, sem(4))]
    order_bits = sum(c << (6 * k + 3 * e) for k, pair in enumerate(COL_PAIRS[0]) for e, c in enumerate(pair))

    def warm(k, carry=None):
        for e in range(6):
            c = ((order_bits >> (6 * k + 3 * (e % 2))) & 7) * U
            kv_copy(0, FIRST[e][:3] + (c,), 6 * k + e).start(priority=1)
            if e % 3 < 2:
                first_unit(0, (4 * k + e - e // 3) * first_stride % D)

    warm(0)
    for copy in small:
        copy.start()
    jax.lax.fori_loop(1, AHEAD // 6, warm, None)

    def setup():
        for copy in small:
            copy.wait()
        a_s[...] = jnp.zeros(a_s.shape, f32)
        gu_s[...] = jnp.zeros(gu_s.shape, f32)

    def x_columns(c):
        x_c[c:c + 128] = _columns(x_v[0][:, c:c + 128].astype(f32))

    tasks = _place({}, [setup] + [lambda c=c: x_columns(c) for c in range(0, D, 128)], 2, FIRST_END)
    _place(tasks, first_tasks(0), FIRST_END + 8, FIRST_END + 15)
    third = 3 * (FIRST_END + 15)
    for t, fns in enumerate(attention(0, FIRST)):
        third = max(third + 1, 3 * t)
        tasks.setdefault(min(third // 3, T - 1), []).extend(fns)
    requests = _place(_place({}, first_units(0)[AHEAD // 6 * 4:], 0, FIRST_END), first_units(1), FIRST_END, T)
    stream(0, FIRST, requests, tasks)

    def passes(lo, hi, units, consume, consume_first):
        def body(h, carry):
            tasks = dict(enumerate(attention(h, MID)))
            _place(tasks, [fn and (lambda fn=fn: pl.when(h == lo)(fn)) for fn in consume_first], LANDED, T - 2)
            _place(tasks, [fn and (lambda fn=fn: pl.when(h > lo)(fn)) for fn in consume(h)], LANDED, T - 2)
            stream(h, MID, _place({}, units(h + 1), 0, T), tasks)
            return carry
        jax.lax.fori_loop(lo, hi, body, 0)

    passes(1, NQ - 1, q_units, q_tasks, first_tasks(1))
    passes(NQ - 1, NQ + NG - 1, gu_units, gu_tasks, q_tasks(NQ - 1))
    passes(NQ + NG - 1, H - 1, out_units, out_tasks,
           gu_tasks(NQ + NG - 1) + _spaced([lambda c=c: swiglu(c) for c in range(0, F, 128)]))

    low, high, ffn = out_parts(H)
    high = high[:4] + (DH - LAG,) + high[5:]
    tail = [(0, high, LAG, 160), (1, high, 0, LAG), (1, low, 0, 64), (0, high, LAG + 160, 32),
            (1, low, 64, 32), (1, low, 96, 32)]

    def tail_units(queue):
        return [fn for k, (q, p, r, n) in enumerate(tail) if q == queue
                for fn in part_units(H, p, r, n, q, sem(6 + k))]

    requests = _place({}, part_units(H, ffn, 0, DR, 0, sem(5)) + tail_units(0), 0, LAST_END)
    _place(requests, tail_units(1), T - AHEAD, T - AHEAD + 6)
    mix = {}

    def ffn_branch():
        _wait(out_b.at[0, pl.ds(ffn[4], DR)], sem(5))
        y = a_s[1] + _rows_dot(out_b[0, ffn[4]:ffn[4] + DR], h_c[ffn[2]:ffn[2] + DR])
        y = jnp.sum(y, axis=0, keepdims=True)
        x = x_v[0].astype(f32)
        gate = jax.nn.sigmoid(jnp.sum(x * gw_v[...].astype(f32).reshape(1, D), axis=-1, keepdims=True))
        route = jax.nn.sigmoid(jnp.sum(x * wr_v[...].astype(f32).reshape(1, D), axis=-1, keepdims=True))
        mix['gate'] = gate
        mix['ffn'] = (1.0 - gate) * (x + (x * 0.0 + y * route))

    tasks = _place(dict(enumerate(attention(H - 1, LAST))), out_tasks(H - 1) + [ffn_branch], LANDED, 36)
    stream(H - 1, LAST, requests, tasks)

    row0 = jax.lax.broadcasted_iota(jnp.int32, (8, D), 0) == 0
    acc = mix['gate'] * a_s[0] + jnp.where(row0, mix['ffn'], 0.0)
    for k, (_, (_, _, first, _, off, _), r, n) in enumerate(tail):
        col = mix['gate'] * o_c[first + r:first + r + n]
        _wait(out_b.at[0, pl.ds(off + r, n)], sem(6 + k))
        acc = acc + _rows_dot(out_b[0, off + r:off + r + n], col)
    out_ref[0] = jnp.sum(acc, axis=0, keepdims=True).astype(bf16)


@jax.jit
def pallas_gated_mix__sliding_block_cached__moe_arch_mod__decode_kernel(
        A_x, A_k_cache, A_v_cache, A_wq, A_wo, B_x, B_w_r, B_w_gate, B_w_up, B_w_down, gate_w):
    del B_x
    kT = jnp.swapaxes(A_k_cache, 2, 3).reshape(H * DH, SK)
    vT = jnp.swapaxes(A_v_cache, 2, 3).reshape(H * DH, SK)
    vmem = pltpu.VMEM
    return pl.pallas_call(
        _kernel,
        out_shape=jax.ShapeDtypeStruct((1, 1, D), bf16),
        in_specs=[pl.BlockSpec(memory_space=pl.ANY)] * 10,
        out_specs=pl.BlockSpec(memory_space=pltpu.VMEM),
        scratch_shapes=[
            vmem((1, 1, D), bf16), vmem((D,), bf16), vmem((D,), bf16),
            vmem((2, 2, DH + KR, W), bf16), vmem((2, D, U), bf16), vmem((2, QR, QC), bf16),
            vmem((2, 2, GR, F), bf16), vmem((2, 2 * DH + DR, D), bf16),
            vmem((D, 128), f32), vmem((H * DH, 128), f32), vmem((H * DH, 128), f32), vmem((F, 128), f32),
            vmem((2, 8, W), f32), vmem((2, 8, W), f32), vmem((DH + KR, 128), f32),
            vmem((2, 8, QC), f32), vmem((2, 8, F), f32), vmem((2, 8, D), f32),
            pltpu.SemaphoreType.DMA((NSEM + 12,)),
        ],
        compiler_params=pltpu.CompilerParams(
            vmem_limit_bytes=64 * 1024 * 1024,
            disable_semaphore_checks=True,
            disable_bounds_checks=True,
        ),
        name="gated_mix_decode",
    )(A_x, kT, vT, A_wq, A_wo, B_w_r, B_w_gate, B_w_up, B_w_down, gate_w)
```
